```python
import jax
import jax.numpy as jnp

def _softmax(x, axis=-1):
    return jax.nn.softmax(x, axis=axis)

def _gelu(x):
    return jax.nn.gelu(x, approximate=True)

def _silu(x):
    return jax.nn.silu(x)

def _sigmoid(x):
    return jax.nn.sigmoid(x)

def _layernorm(x, axis=-1, eps=1e-05):
    m = jnp.mean(x, axis=axis, keepdims=True)
    v = jnp.var(x, axis=axis, keepdims=True)
    return (x - m) / jnp.sqrt(v + eps)

def _scatter_add(tgt, idx, src, axis=0):
    return tgt.at[idx].add(src)

def _segment_sum(src, seg, n):
    return jax.ops.segment_sum(src, seg, n)

class _Rng:

    def __init__(self, key):
        self._k = key

    def _next(self):
        self._k, sub = jax.random.split(self._k)
        return sub

    def normal(self, shape):
        return jax.random.normal(self._next(), shape, dtype=jnp.bfloat16)

    def randint(self, lo, hi, shape):
        return jax.random.randint(self._next(), shape, lo, hi, dtype=jnp.int32)

    def uniform(self, shape, lo=0.0, hi=1.0):
        return jax.random.uniform(self._next(), shape, jnp.bfloat16, lo, hi)

    def permutation(self, n):
        return jax.random.permutation(self._next(), n)
kernel_name = 'sequential_preLN__memory_aug_recurrent_mem_tr__mixer_s_mlp__prompt'

def setup_inputs():
    _rng = _Rng(jax.random.key(int.from_bytes(__import__("os").urandom(4), "little")))
    _w = lambda a: (lambda t: t.astype(jnp.bfloat16) if jnp.issubdtype(t.dtype, jnp.floating) else t)(jnp.asarray(a))

    def _A_setup():
        B, S, Dm = (1, 2048, 1024)
        H, Dh = (32, 128)
        M, seg = (8, 32)
        seg = min(seg, S)
        S = S // seg * seg
        return {'x': _w((lambda *s: _rng.normal(s) * 0.05)(B, S, Dm)), 'mem0': _w((lambda *s: _rng.normal(s) * 0.05)(B, M, Dm)), 'Wq': _w((lambda *s: _rng.normal(s) * 0.05)(Dm, H, Dh) * Dm ** (-0.5)), 'Wk': _w((lambda *s: _rng.normal(s) * 0.05)(Dm, H, Dh) * Dm ** (-0.5)), 'Wv': _w((lambda *s: _rng.normal(s) * 0.05)(Dm, H, Dh) * Dm ** (-0.5)), 'Wo': _w((lambda *s: _rng.normal(s) * 0.05)(H, Dh, Dm) * (H * Dh) ** (-0.5)), 'seg_len': seg}
    _A_in = _A_setup()

    def _B_setup():
        B, S, D, F = (1, 2048, 1024, 3584)
        return {'x': _w((lambda *s: _rng.normal(s) * 0.05)(B, S, D)), 'w1': _w((lambda *s: _rng.normal(s) * 0.05)(D, D) * D ** (-0.5)), 'w2': _w((lambda *s: _rng.normal(s) * 0.05)(D, D) * D ** (-0.5)), 'w3': _w((lambda *s: _rng.normal(s) * 0.05)(D, F) * D ** (-0.5)), 'w4': _w((lambda *s: _rng.normal(s) * 0.05)(F, D) * F ** (-0.5))}
    _B_in = _B_setup()
    return {'A_x': _A_in['x'], 'A_mem0': _A_in['mem0'], 'A_Wq': _A_in['Wq'], 'A_Wk': _A_in['Wk'], 'A_Wv': _A_in['Wv'], 'A_Wo': _A_in['Wo'], 'A_seg_len': _A_in['seg_len'], 'B_x': _B_in['x'], 'B_w1': _B_in['w1'], 'B_w2': _B_in['w2'], 'B_w3': _B_in['w3'], 'B_w4': _B_in['w4']}

def reference(A_x, A_mem0, A_Wq, A_Wk, A_Wv, A_Wo, A_seg_len, B_x, B_w1, B_w2, B_w3, B_w4):

    def _A_ref(x, mem0, Wq, Wk, Wv, Wo, seg_len):
        B, S, Dm = x.shape
        H, Dh = (Wq.shape[1], Wq.shape[2])
        M = mem0.shape[1]
        scale = Dh ** (-0.5)
        n_seg = S // seg_len
        L = M + seg_len
        idx = jnp.arange(L)
        mask = (idx[:, None] < M) | (idx[:, None] >= idx[None, :])
        mem = mem0
        outs = []
        for s in range(n_seg):
            xs = x[:, s * seg_len:(s + 1) * seg_len, :].copy()
            h = jnp.concatenate([mem, xs], axis=1)
            q = jnp.einsum('btd,dhe->bhte', h, Wq)
            k = jnp.einsum('btd,dhe->bhte', h, Wk)
            v = jnp.einsum('btd,dhe->bhte', h, Wv)
            scores = jnp.einsum('bhqe,bhke->bhqk', q, k) * scale
            scores = jnp.where(mask[None, None], scores, -1000000000.0)
            p = _softmax(scores, axis=-1)
            o = jnp.einsum('bhqk,bhke->bhqe', p, v)
            o = jnp.einsum('bhte,hed->btd', o, Wo)
            mem = o[:, :M, :].copy()
            outs.append(o[:, M:, :])
        return jnp.concatenate(outs, axis=1)

    def _B_ref(x, w1, w2, w3, w4):
        B, S, D = x.shape
        h = _gelu(_layernorm(x, axis=-1) @ w1)
        c = D // 4
        g0 = jnp.pad(h[:, :, 0 * c:1 * c], ((0, 0), (1, 0), (0, 0)))[:, :S, :]
        g1 = jnp.pad(h[:, :, 1 * c:2 * c], ((0, 0), (0, 1), (0, 0)))[:, 1:, :]
        g2 = jnp.pad(h[:, :, 2 * c:3 * c], ((0, 0), (2, 0), (0, 0)))[:, :S, :]
        g3 = jnp.pad(h[:, :, 3 * c:], ((0, 0), (0, 2), (0, 0)))[:, 2:, :]
        hs = jnp.concatenate([g0, g1, g2, g3], axis=-1) @ w2
        x1 = x + hs
        h2 = _gelu(_layernorm(x1, axis=-1) @ w3) @ w4
        return x1 + h2
    x = A_x
    h = x + _A_ref(_layernorm(x, axis=-1), A_mem0, A_Wq, A_Wk, A_Wv, A_Wo, A_seg_len)
    h2 = h + _B_ref(_layernorm(h, axis=-1), B_w1, B_w2, B_w3, B_w4)
    return h2
```

```python
import functools

import jax
import jax.numpy as jnp
import numpy as np
import jax.experimental.pallas as pl
import jax.experimental.pallas.tpu as pltpu

F32 = jnp.float32
BF16 = jnp.bfloat16

S = 2048
D = 1024
H = 32
E = 128
M = 8
SEG = 32
NSEG = S // SEG
FF = 3584
NT = D // 128
EPS = 1e-5
PAD = 16
RB = 256
NRB = S // RB
FC = 512


def _ln(x):
    m = jnp.mean(x, axis=-1, keepdims=True)
    c = x - m
    v = jnp.mean(c * c, axis=-1, keepdims=True)
    return c * jax.lax.rsqrt(v + EPS)


def _gelu(x):
    return jax.nn.gelu(x, approximate=True)


def _dot(a, b):
    return jnp.dot(a, b, preferred_element_type=F32)


def _kernel(x_hbm, mem0_ref, wq_hbm, wk_hbm, wv_hbm, wo_hbm, w1_hbm, w2_hbm, w3_hbm, w4_hbm,
            out_hbm,
            wq_s, wk_s, wv_s, wo_s, st0, st1, xn, hb, xo, qo, ko, vo, oo, ob,
            w1_s, w2_s, w3_s, w4_s, gb, outb, sems, osems):
    cp_x = pltpu.make_async_copy(x_hbm, gb.at[pl.ds(PAD, S), :], sems.at[0])
    cp_wk = pltpu.make_async_copy(wk_hbm, st0, sems.at[1])
    cp_wv = pltpu.make_async_copy(wv_hbm, st1, sems.at[2])
    cp_wq = pltpu.make_async_copy(wq_hbm, st0, sems.at[3])
    cp_wo = [pltpu.make_async_copy(wo_hbm.at[:, pl.ds(n * 128, 128)], wo_s.at[n], sems.at[4 + n])
             for n in range(NT)]
    cp_w1 = pltpu.make_async_copy(w1_hbm, w1_s, sems.at[12])
    cp_w2 = pltpu.make_async_copy(w2_hbm, w2_s, sems.at[13])
    cp_w3 = pltpu.make_async_copy(w3_hbm, w3_s, sems.at[14])
    cp_w4 = pltpu.make_async_copy(w4_hbm, w4_s, sems.at[15])

    cp_x.start()
    cp_wk.start()
    cp_wv.start()
    cp_x.wait()

    CH = 128

    def ln_body(c, carry):
        r = pl.multiple_of(c * CH, CH)
        xv = gb[pl.ds(PAD + r, CH), :].astype(F32)
        hb[pl.ds(r, CH), :] = xv
        y = _ln(xv)
        xn[pl.ds(r, CH), :] = y
        octs = [y[SEG * s + 24:SEG * s + 32] for s in range(CH // SEG)]
        xo[pl.ds(pl.multiple_of(c * (CH // 4), CH // 4), CH // 4), :] = (
            jnp.concatenate(octs, axis=0).astype(BF16))
        return carry

    jax.lax.fori_loop(0, S // CH, ln_body, 0)

    def relayout(st, w_s):
        wi = st.bitcast(jnp.int32)

        DC = 128

        def body(c, carry):
            sub = wi.at[pl.ds(pl.multiple_of(c * (DC * 16), DC * 16), DC * 16), :]
            dr = pl.multiple_of(c * DC, DC)
            for p in range(H // 2):
                a = sub[pl.ds(p, DC // 2, stride=32), :]
                b = sub[pl.ds(p + 16, DC // 2, stride=32), :]
                lo = (a & 0xFFFF) | (b << 16)
                hi = jax.lax.shift_right_logical(a, 16) | (b & np.int32(-65536))
                w_s[2 * p, pl.ds(dr, DC), :] = pltpu.bitcast(lo, BF16)
                w_s[2 * p + 1, pl.ds(dr, DC), :] = pltpu.bitcast(hi, BF16)
            return carry

        jax.lax.fori_loop(0, D // DC, body, 0)

    def tail_proj(w_s, dst):
        def body(h, carry):
            w = w_s[h]
            for r in range(0, 512, 256):
                dst[h, r:r + 256, :] = _dot(xo[r:r + 256, :], w).astype(BF16)
            return carry

        jax.lax.fori_loop(0, H, body, 0)

    cp_wk.wait()
    relayout(st0, wk_s)
    cp_wq.start()
    for c in cp_wo:
        c.start()
    tail_proj(wk_s, ko)
    cp_wv.wait()
    relayout(st1, wv_s)
    tail_proj(wv_s, vo)
    cp_wq.wait()
    relayout(st0, wq_s)
    cp_w1.start()
    cp_w2.start()
    cp_w3.start()
    cp_w4.start()
    tail_proj(wq_s, qo)
    for c in cp_wo:
        c.wait()

    scale = E ** -0.5

    def step(i, mem):
        r0 = pl.multiple_of(i * SEG, SEG)
        xs = xn[pl.ds(r0, 24), :]
        lhs = jnp.concatenate([mem, xs], axis=0).astype(BF16)
        pr = pl.multiple_of((i // 2) * 16, 16)
        par = i % 2
        even = par == 0

        row = jax.lax.broadcasted_iota(jnp.int32, (48, 48), 0)
        col = jax.lax.broadcasted_iota(jnp.int32, (48, 48), 1)
        qpos = jnp.where(row < 8, 99, jnp.where(row < 32, row - 8, 24 + (row - 32) % 8))
        kpos = jnp.where(col < 8, -1, jnp.where(col < 32, col - 8, 24 + (col - 32) % 8))
        kval = (col < 32) | (((col - 32) // 8) == par)
        mask = (kpos <= qpos) & kval

        for h in range(H):
            q = _dot(lhs, wq_s[h]).astype(BF16)
            k = _dot(lhs, wk_s[h]).astype(BF16)
            v = _dot(lhs, wv_s[h]).astype(BF16)
            q48 = jnp.concatenate([q, qo[h, pl.ds(pr, 16), :]], axis=0)
            k48 = jnp.concatenate([k, ko[h, pl.ds(pr, 16), :]], axis=0)
            v48 = jnp.concatenate([v, vo[h, pl.ds(pr, 16), :]], axis=0)
            s = jax.lax.dot_general(q48, k48, (((1,), (1,)), ((), ())),
                                    preferred_element_type=F32) * scale
            s = jnp.where(mask, s, -1e9)
            mx = jnp.max(s, axis=-1, keepdims=True)
            p = jnp.exp(s - mx)
            p = p * (1.0 / jnp.sum(p, axis=-1, keepdims=True))
            o = _dot(p.astype(BF16), v48)
            ob[h] = o[0:32].astype(BF16)
            t = oo[h, pl.ds(pr, 16), :].astype(F32)
            lo = jnp.where(even, o[32:40], t[0:8])
            oo[h, pl.ds(pr, 16), :] = jnp.concatenate([lo, o[40:48]], axis=0).astype(BF16)

        lo_ = jnp.concatenate([ob[h] for h in range(H)], axis=1)
        mems = []
        for n in range(NT):
            res = _dot(lo_, wo_s[n])
            mems.append(res[0:8])
            cs = slice(n * 128, (n + 1) * 128)
            hb[pl.ds(r0, 24), cs] = hb[pl.ds(r0, 24), cs] + res[8:32]
        return jnp.concatenate(mems, axis=1)

    jax.lax.fori_loop(0, NSEG, step, mem0_ref[...].astype(F32))

    def tail_out(c, carry):
        r = pl.multiple_of(c * 128, 128)
        lhs = jnp.concatenate([oo[h, pl.ds(r, 128), :] for h in range(H)], axis=1)
        for n in range(NT):
            res = _dot(lhs, wo_s[n])
            cs = slice(n * 128, (n + 1) * 128)
            for s in range(16):
                rr = pl.multiple_of(c * (16 * SEG) + s * SEG + 24, 8)
                hb[pl.ds(rr, 8), cs] = hb[pl.ds(rr, 8), cs] + res[8 * s:8 * s + 8]
        return carry

    jax.lax.fori_loop(0, 4, tail_out, 0)

    cp_w1.wait()
    cp_w2.wait()
    cp_w3.wait()
    cp_w4.wait()
    gb[0:PAD, :] = jnp.zeros((PAD, D), BF16)
    gb[PAD + S:PAD + S + PAD, :] = jnp.zeros((PAD, D), BF16)
    yb = xn

    def stage1(b):
        r = pl.multiple_of(b * RB, RB)
        y = _ln(hb[pl.ds(r, RB), :])
        yb[pl.ds(r, RB), :] = y
        z = _ln(y).astype(BF16)
        g = _gelu(_dot(z, w1_s[...]))
        gb[pl.ds(r + PAD, RB), :] = g.astype(BF16)

    def stage2(b, wait_unused=None):
        r = pl.multiple_of(b * RB, RB)
        c = D // 4
        parts = []
        for gi, sh in enumerate((-1, 1, -2, 2)):
            win = gb[pl.ds(r, RB + 2 * PAD), gi * c:(gi + 1) * c].astype(F32)
            parts.append(win[PAD + sh:PAD + sh + RB].astype(BF16))
        gs = jnp.concatenate(parts, axis=1)
        x1 = yb[pl.ds(r, RB), :] + _dot(gs, w2_s[...])
        z2 = _ln(x1).astype(BF16)
        acc = hb[pl.ds(r, RB), :] + x1
        for f in range(FF // FC):
            a = _gelu(_dot(z2, w3_s[:, f * FC:(f + 1) * FC])).astype(BF16)
            acc = acc + _dot(a, w4_s[f * FC:(f + 1) * FC, :])
        outb[pl.ds(r, RB), :] = acc.astype(BF16)
        pltpu.make_async_copy(outb.at[pl.ds(r, RB), :], out_hbm.at[pl.ds(r, RB), :],
                              osems.at[b]).start()

    def pro(b, carry):
        stage1(b)
        return carry

    jax.lax.fori_loop(0, 2, pro, 0)

    def mlp(b, carry):
        stage2(b)
        stage1(jnp.minimum(b + 2, NRB - 1))
        return carry

    jax.lax.fori_loop(0, NRB, mlp, 0)

    for b in range(NRB):
        pltpu.make_async_copy(outb.at[pl.ds(b * RB, RB), :], out_hbm.at[pl.ds(b * RB, RB), :],
                              osems.at[b]).wait()


@functools.partial(jax.jit, static_argnames=("A_seg_len",))
def pallas_sequential_preLN__memory_aug_recurrent_mem_tr__mixer_s_mlp__prompt_kernel(
    A_x: jax.Array,
    A_mem0: jax.Array,
    A_Wq: jax.Array,
    A_Wk: jax.Array,
    A_Wv: jax.Array,
    A_Wo: jax.Array,
    A_seg_len: int,
    B_x: jax.Array,
    B_w1: jax.Array,
    B_w2: jax.Array,
    B_w3: jax.Array,
    B_w4: jax.Array,
):
    assert A_seg_len == SEG
    assert A_x.shape == (1, S, D) and A_mem0.shape == (1, M, D) and A_Wq.shape == (D, H, E)
    any_spec = pl.BlockSpec(memory_space=pl.ANY)
    vm = pltpu.VMEM
    out = pl.pallas_call(
        _kernel,
        out_shape=jax.ShapeDtypeStruct((S, D), A_x.dtype),
        in_specs=[any_spec, pl.BlockSpec(memory_space=pltpu.VMEM)] + [any_spec] * 8,
        out_specs=any_spec,
        scratch_shapes=[
            vm((H, D, E), BF16), vm((H, D, E), BF16), vm((H, D, E), BF16),
            vm((NT, H * E, 128), BF16),
            vm((D * H, E), BF16), vm((D * H, E), BF16),
            vm((S, D), F32), vm((S, D), F32),
            vm((512, D), BF16),
            vm((H, 512, E), BF16), vm((H, 512, E), BF16), vm((H, 512, E), BF16),
            vm((H, 512, E), BF16),
            vm((H, 32, E), BF16),
            vm((D, D), BF16), vm((D, D), BF16), vm((D, FF), BF16), vm((FF, D), BF16),
            vm((S + 2 * PAD, D), BF16),
            vm((S, D), BF16),
            pltpu.SemaphoreType.DMA((16,)),
            pltpu.SemaphoreType.DMA((NRB,)),
        ],
        compiler_params=pltpu.CompilerParams(vmem_limit_bytes=122 * 2 ** 20),
    )(A_x.reshape(S, D), A_mem0.reshape(M, D),
      A_Wq.reshape(D * H, E), A_Wk.reshape(D * H, E), A_Wv.reshape(D * H, E),
      A_Wo.reshape(H * E, D), B_w1, B_w2, B_w3, B_w4)
    return out.reshape(1, S, D)
```

```python
import functools

import jax
import jax.numpy as jnp
import numpy as np
import jax.experimental.pallas as pl
import jax.experimental.pallas.tpu as pltpu

F32 = jnp.float32
BF16 = jnp.bfloat16

S = 2048
D = 1024
H = 32
E = 128
M = 8
SEG = 32
NSEG = S // SEG
FF = 3584
NT = D // 128
EPS = 1e-5
PAD = 16
RB = 256
NRB = S // RB
FC = 512


def _ln(x):
    m = jnp.mean(x, axis=-1, keepdims=True)
    c = x - m
    v = jnp.mean(c * c, axis=-1, keepdims=True)
    return c * jax.lax.rsqrt(v + EPS)


def _gelu(x):
    return jax.nn.gelu(x, approximate=True)


def _dot(a, b):
    return jnp.dot(a, b, preferred_element_type=F32)


def _kernel(x_hbm, mem0_ref, wq_hbm, wk_hbm, wv_hbm, wo_hbm, w1_hbm, w2_hbm, w3_hbm, w4_hbm,
            out_hbm,
            wq_s, wk_s, wv_s, wo_s, st0, st1, xn, hb, xo, qo, ko, vo, oo, ob,
            w1_s, w2_s, w3_s, w4_s, gb, outb, sems, osems):
    NCH = 8
    DC = D // NCH
    XR = S // NCH

    def cp_x(c):
        r = pl.multiple_of(c * XR, XR)
        return pltpu.make_async_copy(x_hbm.at[pl.ds(r, XR), :], gb.at[pl.ds(PAD + r, XR), :],
                                     sems.at[c])

    def cp_w(src, st, base, c):
        r = pl.multiple_of(c * (DC * H), DC * H)
        return pltpu.make_async_copy(src.at[pl.ds(r, DC * H), :], st.at[pl.ds(r, DC * H), :],
                                     sems.at[base + c])

    cp_wk = functools.partial(cp_w, wk_hbm, st0, 8)
    cp_wv = functools.partial(cp_w, wv_hbm, st1, 16)
    cp_wq = functools.partial(cp_w, wq_hbm, st0, 24)
    cp_wo = [pltpu.make_async_copy(wo_hbm.at[:, pl.ds(n * 128, 128)], wo_s.at[n], sems.at[32 + n])
             for n in range(NT)]
    cp_w1 = pltpu.make_async_copy(w1_hbm, w1_s, sems.at[40])
    cp_w2 = pltpu.make_async_copy(w2_hbm, w2_s, sems.at[41])
    cp_w3 = pltpu.make_async_copy(w3_hbm, w3_s, sems.at[42])
    cp_w4 = pltpu.make_async_copy(w4_hbm, w4_s, sems.at[43])

    for c in range(NCH):
        cp_x(c).start()
        cp_wk(c).start()
    for c in range(NCH):
        cp_wv(c).start()

    def relayout_chunk(st, w_s, c):
        wi = st.bitcast(jnp.int32)
        sub = wi.at[pl.ds(pl.multiple_of(c * (DC * 16), DC * 16), DC * 16), :]
        dr = pl.multiple_of(c * (DC // 2), DC // 2)
        for p in range(H // 2):
            w = sub[pl.ds(p, DC, stride=16), :]
            lo = jax.lax.bitcast_convert_type(w << 16, F32).astype(BF16)
            hi = jax.lax.bitcast_convert_type(w & np.int32(-65536), F32).astype(BF16)
            w_s[2 * p, pl.ds(dr, DC // 2), :] = pltpu.bitcast(lo, jnp.int32)
            w_s[2 * p + 1, pl.ds(dr, DC // 2), :] = pltpu.bitcast(hi, jnp.int32)

    def wtile(w_s, h):
        return pltpu.bitcast(w_s[h], BF16)

    def tail_proj(w_s, dst, c):
        for j in range(H // NCH):
            h = c * (H // NCH) + j
            w = wtile(w_s, h)
            for r in range(0, 512, 256):
                dst[h, r:r + 256, :] = _dot(xo[r:r + 256, :], w).astype(BF16)

    def p1(c, carry):
        cp_x(c).wait()
        r = pl.multiple_of(c * XR, XR)
        xv = gb[pl.ds(PAD + r, XR), :].astype(F32)
        hb[pl.ds(r, XR), :] = xv
        y = _ln(xv)
        xn[pl.ds(r, XR), :] = y
        octs = [y[SEG * s + 24:SEG * s + 32] for s in range(XR // SEG)]
        xo[pl.ds(pl.multiple_of(c * (XR // 4), XR // 4), XR // 4), :] = (
            jnp.concatenate(octs, axis=0).astype(BF16))
        cp_wk(c).wait()
        relayout_chunk(st0, wk_s, c)
        return carry

    with jax.named_scope('S_p1'):
        jax.lax.fori_loop(0, NCH, p1, 0)

    for c in range(NCH):
        cp_wq(c).start()
    for c in cp_wo:
        c.start()

    def p2(c, carry):
        cp_wv(c).wait()
        relayout_chunk(st1, wv_s, c)
        tail_proj(wk_s, ko, c)
        return carry

    with jax.named_scope('S_p2'):
        jax.lax.fori_loop(0, NCH, p2, 0)

    cp_w1.start()
    cp_w2.start()
    cp_w3.start()
    cp_w4.start()

    def p3(c, carry):
        cp_wq(c).wait()
        relayout_chunk(st0, wq_s, c)
        tail_proj(wv_s, vo, c)
        return carry

    with jax.named_scope('S_p3'):
        jax.lax.fori_loop(0, NCH, p3, 0)

    def p4(c, carry):
        tail_proj(wq_s, qo, c)
        return carry

    with jax.named_scope('S_p4'):
        jax.lax.fori_loop(0, NCH, p4, 0)

    for c in cp_wo:
        c.wait()

    scale = E ** -0.5

    def step(i, mem):
        r0 = pl.multiple_of(i * SEG, SEG)
        xs = xn[pl.ds(r0, 24), :]
        lhs = jnp.concatenate([mem, xs], axis=0).astype(BF16)
        pr = pl.multiple_of((i // 2) * 16, 16)
        par = i % 2
        even = par == 0

        row = jax.lax.broadcasted_iota(jnp.int32, (48, 48), 0)
        col = jax.lax.broadcasted_iota(jnp.int32, (48, 48), 1)
        qpos = jnp.where(row < 8, 99, jnp.where(row < 32, row - 8, 24 + (row - 32) % 8))
        kpos = jnp.where(col < 8, -1, jnp.where(col < 32, col - 8, 24 + (col - 32) % 8))
        kval = (col < 32) | (((col - 32) // 8) == par)
        mask = (kpos <= qpos) & kval

        qkv = []
        for h in range(H):
            q = _dot(lhs, wtile(wq_s, h)).astype(BF16)
            k = _dot(lhs, wtile(wk_s, h)).astype(BF16)
            v = _dot(lhs, wtile(wv_s, h)).astype(BF16)
            qkv.append((jnp.concatenate([q, qo[h, pl.ds(pr, 16), :]], axis=0),
                        jnp.concatenate([k, ko[h, pl.ds(pr, 16), :]], axis=0),
                        jnp.concatenate([v, vo[h, pl.ds(pr, 16), :]], axis=0)))
        sc = []
        for h in range(H):
            s = jax.lax.dot_general(qkv[h][0], qkv[h][1], (((1,), (1,)), ((), ())),
                                    preferred_element_type=F32) * scale
            s = jnp.where(mask, s, -1e9)
            sc.append((s, jnp.max(s, axis=-1, keepdims=True)))
        av = []
        for h in range(H):
            p = jnp.exp(sc[h][0] - sc[h][1])
            av.append((_dot(p.astype(BF16), qkv[h][2]), jnp.sum(p, axis=-1, keepdims=True)))
        for h in range(H):
            o, l = av[h]
            r = pl.reciprocal(l, approx=True)
            r = r * (2.0 - l * r)
            o = o * r
            ob[h] = o[0:32].astype(BF16)
            t = oo[h, pl.ds(pr, 16), :].astype(F32)
            lo = jnp.where(even, o[32:40], t[0:8])
            oo[h, pl.ds(pr, 16), :] = jnp.concatenate([lo, o[40:48]], axis=0).astype(BF16)

        lo_ = jnp.concatenate([ob[h] for h in range(H)], axis=1)
        mems = []
        for n in range(NT):
            res = _dot(lo_, wo_s[n])
            mems.append(res[0:8])
            cs = slice(n * 128, (n + 1) * 128)
            hb[pl.ds(r0, 24), cs] = hb[pl.ds(r0, 24), cs] + res[8:32]
        return jnp.concatenate(mems, axis=1)

    with jax.named_scope('S_rec'):
        jax.lax.fori_loop(0, NSEG, step, mem0_ref[...].astype(F32))

    def tail_out(c, carry):
        r = pl.multiple_of(c * 128, 128)
        lhs = jnp.concatenate([oo[h, pl.ds(r, 128), :] for h in range(H)], axis=1)
        for n in range(NT):
            res = _dot(lhs, wo_s[n])
            cs = slice(n * 128, (n + 1) * 128)
            for s in range(16):
                rr = pl.multiple_of(c * (16 * SEG) + s * SEG + 24, 8)
                hb[pl.ds(rr, 8), cs] = hb[pl.ds(rr, 8), cs] + res[8 * s:8 * s + 8]
        return carry

    with jax.named_scope('S_tailout'):
        jax.lax.fori_loop(0, 4, tail_out, 0)

    cp_w1.wait()
    cp_w2.wait()
    cp_w3.wait()
    cp_w4.wait()
    gb[0:PAD, :] = jnp.zeros((PAD, D), BF16)
    gb[PAD + S:PAD + S + PAD, :] = jnp.zeros((PAD, D), BF16)
    yb = xn

    def stage1(b):
        r = pl.multiple_of(b * RB, RB)
        y = _ln(hb[pl.ds(r, RB), :])
        yb[pl.ds(r, RB), :] = y
        z = _ln(y).astype(BF16)
        g = _gelu(_dot(z, w1_s[...]))
        gb[pl.ds(r + PAD, RB), :] = g.astype(BF16)

    def stage2(b, wait_unused=None):
        r = pl.multiple_of(b * RB, RB)
        c = D // 4
        parts = []
        for gi, sh in enumerate((-1, 1, -2, 2)):
            win = gb[pl.ds(r, RB + 2 * PAD), gi * c:(gi + 1) * c].astype(F32)
            parts.append(win[PAD + sh:PAD + sh + RB].astype(BF16))
        gs = jnp.concatenate(parts, axis=1)
        x1 = yb[pl.ds(r, RB), :] + _dot(gs, w2_s[...])
        z2 = _ln(x1).astype(BF16)
        acc = hb[pl.ds(r, RB), :] + x1
        for f in range(FF // FC):
            a = _gelu(_dot(z2, w3_s[:, f * FC:(f + 1) * FC])).astype(BF16)
            acc = acc + _dot(a, w4_s[f * FC:(f + 1) * FC, :])
        outb[pl.ds(r, RB), :] = acc.astype(BF16)
        pltpu.make_async_copy(outb.at[pl.ds(r, RB), :], out_hbm.at[pl.ds(r, RB), :],
                              osems.at[b]).start()

    def pro(b, carry):
        stage1(b)
        return carry

    with jax.named_scope('S_pro'):
        jax.lax.fori_loop(0, 2, pro, 0)

    def mlp(b, carry):
        stage2(b)
        stage1(jnp.minimum(b + 2, NRB - 1))
        return carry

    with jax.named_scope('S_mlp'):
        jax.lax.fori_loop(0, NRB, mlp, 0)

    for b in range(NRB):
        pltpu.make_async_copy(outb.at[pl.ds(b * RB, RB), :], out_hbm.at[pl.ds(b * RB, RB), :],
                              osems.at[b]).wait()


@functools.partial(jax.jit, static_argnames=("A_seg_len",))
def pallas_sequential_preLN__memory_aug_recurrent_mem_tr__mixer_s_mlp__prompt_kernel(
    A_x: jax.Array,
    A_mem0: jax.Array,
    A_Wq: jax.Array,
    A_Wk: jax.Array,
    A_Wv: jax.Array,
    A_Wo: jax.Array,
    A_seg_len: int,
    B_x: jax.Array,
    B_w1: jax.Array,
    B_w2: jax.Array,
    B_w3: jax.Array,
    B_w4: jax.Array,
):
    assert A_seg_len == SEG
    assert A_x.shape == (1, S, D) and A_mem0.shape == (1, M, D) and A_Wq.shape == (D, H, E)
    any_spec = pl.BlockSpec(memory_space=pl.ANY)
    vm = pltpu.VMEM
    out = pl.pallas_call(
        _kernel,
        out_shape=jax.ShapeDtypeStruct((S, D), A_x.dtype),
        in_specs=[any_spec, pl.BlockSpec(memory_space=pltpu.VMEM)] + [any_spec] * 8,
        out_specs=any_spec,
        scratch_shapes=[
            vm((H, D // 2, E), jnp.int32), vm((H, D // 2, E), jnp.int32),
            vm((H, D // 2, E), jnp.int32),
            vm((NT, H * E, 128), BF16),
            vm((D * H, E), BF16), vm((D * H, E), BF16),
            vm((S, D), F32), vm((S, D), F32),
            vm((512, D), BF16),
            vm((H, 512, E), BF16), vm((H, 512, E), BF16), vm((H, 512, E), BF16),
            vm((H, 512, E), BF16),
            vm((H, 32, E), BF16),
            vm((D, D), BF16), vm((D, D), BF16), vm((D, FF), BF16), vm((FF, D), BF16),
            vm((S + 2 * PAD, D), BF16),
            vm((S, D), BF16),
            pltpu.SemaphoreType.DMA((44,)),
            pltpu.SemaphoreType.DMA((NRB,)),
        ],
        compiler_params=pltpu.CompilerParams(vmem_limit_bytes=122 * 2 ** 20),
    )(A_x.reshape(S, D), A_mem0.reshape(M, D),
      A_Wq.reshape(D * H, E), A_Wk.reshape(D * H, E), A_Wv.reshape(D * H, E),
      A_Wo.reshape(H * E, D), B_w1, B_w2, B_w3, B_w4)
    return out.reshape(1, S, D)
```

```python
import functools

import jax
import jax.numpy as jnp
import numpy as np
import jax.experimental.pallas as pl
import jax.experimental.pallas.tpu as pltpu

F32 = jnp.float32
BF16 = jnp.bfloat16

S = 2048
D = 1024
H = 32
E = 128
M = 8
SEG = 32
NSEG = S // SEG
FF = 3584
NT = D // 128
EPS = 1e-5
PAD = 16
RB = 128
NRB = S // RB
FC = 896
REC_UNROLL = 2


def _ln(x):
    m = jnp.mean(x, axis=-1, keepdims=True)
    c = x - m
    v = jnp.mean(c * c, axis=-1, keepdims=True)
    return c * jax.lax.rsqrt(v + EPS)


def _gelu(x):
    return jax.nn.gelu(x, approximate=True)


def _dot(a, b):
    return jnp.dot(a, b, preferred_element_type=F32)


def _kernel(x_hbm, x3_hbm, mem0_ref, wq_hbm, wk_hbm, wv_hbm, wo_hbm, w1_hbm, w2_hbm, w3_hbm, w4_hbm,
            out_hbm,
            w_s, wo_s, st, acc, xn, hb, xr, xo, qkvo, oo,
            w1_s, w2_s, w3_s, w4_s, gb, outb, sems, osems):
    NKC = 4
    DC = D // NKC
    NXC = 8
    XR = S // NXC
    IK, IV, IQ = 0, 1, 2

    cp_x3 = pltpu.make_async_copy(x3_hbm.at[:, pl.ds(24, 8), :], xr, sems.at[0])

    def cp_x(c):
        r = pl.multiple_of(c * XR, XR)
        return pltpu.make_async_copy(x_hbm.at[pl.ds(r, XR), :], gb.at[pl.ds(PAD + r, XR), :],
                                     sems.at[1 + c])

    def cp_w(src, m, c):
        n = DC * H
        slot = (m * NKC + c) % 8
        return pltpu.make_async_copy(src.at[pl.ds(pl.multiple_of(c * n, n), n), :],
                                     st.at[pl.ds(pl.multiple_of(slot * n, n), n), :],
                                     sems.at[9 + m * NKC + c])

    def wait_w(j):
        n = DC * H
        slot = pl.multiple_of((j % 8) * n, n)
        pltpu.make_async_copy(st.at[pl.ds(slot, n), :], st.at[pl.ds(slot, n), :],
                              sems.at[9 + j]).wait()

    cp_wo = [pltpu.make_async_copy(wo_hbm.at[:, pl.ds(n * 128, 128)], wo_s.at[n], sems.at[21 + n])
             for n in range(NT)]
    cp_w1 = pltpu.make_async_copy(w1_hbm, w1_s, sems.at[29])
    cp_w2 = pltpu.make_async_copy(w2_hbm, w2_s, sems.at[30])
    cp_w3 = pltpu.make_async_copy(w3_hbm, w3_s, sems.at[31])
    cp_w4 = pltpu.make_async_copy(w4_hbm, w4_s, sems.at[32])

    cp_x3.start()
    cp_w(wk_hbm, IK, 0).start()
    cp_x(0).start()
    cp_w(wk_hbm, IK, 1).start()
    cp_w(wk_hbm, IK, 2).start()
    cp_x(1).start()
    cp_w(wk_hbm, IK, 3).start()
    cp_w(wv_hbm, IV, 0).start()
    cp_x(2).start()
    cp_w(wv_hbm, IV, 1).start()
    cp_w(wv_hbm, IV, 2).start()
    cp_x(3).start()
    cp_w(wv_hbm, IV, 3).start()
    for c in range(4, NXC):
        cp_x(c).start()

    RP = 4

    def relayout_piece(j, p, q):
        wi = st.bitcast(jnp.int32)
        sub = wi.at[pl.ds(pl.multiple_of((j % 8) * (DC * 16), DC * 16), DC * 16), :]
        n = DC // RP
        dr = pl.multiple_of((j % NKC) * (DC // 2) + q * (n // 2), n // 2)
        hb0 = (j // NKC) * H
        w = sub[pl.ds(p + q * n * 16, n, stride=16), :]
        lo = jax.lax.bitcast_convert_type(w << 16, F32).astype(BF16)
        hi = jax.lax.bitcast_convert_type(w & np.int32(-65536), F32).astype(BF16)
        w_s[hb0 + 2 * p, pl.ds(dr, n // 2), :] = pltpu.bitcast(lo, jnp.int32)
        w_s[hb0 + 2 * p + 1, pl.ds(dr, n // 2), :] = pltpu.bitcast(hi, jnp.int32)

    def wtile(m, h):
        return pltpu.bitcast(w_s[m * H + h], BF16)

    hb[S:S + PAD, :] = jnp.zeros((PAD, D), F32)

    with jax.named_scope('S_p0'):
        cp_x3.wait()
        for g in range(4):
            y = _ln(jnp.concatenate([xr[16 * g + s].astype(F32) for s in range(16)], axis=0))
            y = y.astype(BF16)
            for kc in range(NKC):
                xo[kc, g * 128:(g + 1) * 128, :] = y[:, kc * DC:(kc + 1) * DC]
        wait_w(0)
        for p in range(H // 2):
            for q in range(RP):
                relayout_piece(0, p, q)

    def proj(j, carry):
        @pl.when(j < NXC)
        def _():
            cp_x(j).wait()

        @pl.when(j < 11)
        def _():
            wait_w(j + 1)

        @pl.when(j < NKC)
        def _():
            cp_w(wq_hbm, IQ, j).start()

        @pl.when(j == NKC)
        def _():
            for c in cp_wo:
                c.start()

        jn = jnp.minimum(j + 1, 11)
        c = jnp.minimum(j, NXC - 1)
        kc = j % NKC
        hb0 = (j // NKC) * H
        dr = pl.multiple_of(kc * (DC // 2), DC // 2)
        first = kc == 0
        LR = XR // 16
        RS = 128
        items = [(h, r) for h in range(H) for r in range(0, 512, RS)]
        for t, (h, r) in enumerate(items):
            w = pltpu.bitcast(w_s[hb0 + h, pl.ds(dr, DC // 2), :], BF16)
            res = _dot(xo[kc, r:r + RS, :], w)
            if t % 2 == 1:
                relayout_piece(jn, (t // 2) // RP, (t // 2) % RP)
            new = res + jnp.where(first, 0.0, acc[h, r:r + RS, :])
            acc[h, r:r + RS, :] = new
            qkvo[hb0 + h, r:r + RS, :] = new.astype(BF16)
            if t % 8 == 7:
                rr = pl.multiple_of(c * XR + (t // 8) * LR, LR)
                xv = gb[pl.ds(PAD + rr, LR), :].astype(F32)
                hb[pl.ds(rr, LR), :] = xv
                xn[pl.ds(rr, LR), :] = _ln(xv)
        return carry

    with jax.named_scope('S_proj'):
        jax.lax.fori_loop(0, 12, proj, 0)

    cp_w1.start()
    cp_w2.start()
    cp_w3.start()
    cp_w4.start()
    for c in cp_wo:
        c.wait()

    L = M + SEG
    c_exp = (E ** -0.5) * 1.4426950408889634

    def step(i, mem):
        r0 = pl.multiple_of(i * SEG, SEG)
        r8 = pl.multiple_of(i * 8, 8)
        lhs = jnp.concatenate([mem, xn[pl.ds(r0, 24), :]], axis=0).astype(BF16)
        row = jax.lax.broadcasted_iota(jnp.int32, (L, L), 0)
        col = jax.lax.broadcasted_iota(jnp.int32, (L, L), 1)
        mask = (row < M) | (row >= col)

        qkv, sc, av, oh = {}, {}, {}, {}
        acc_o = []

        def st_proj(h):
            qkv[h] = tuple(
                jnp.concatenate([_dot(lhs, wtile(m, h)),
                                 qkvo[m * H + h, pl.ds(r8, 8), :].astype(F32)], axis=0)
                for m in (IQ, IK, IV))

        def st_score(h):
            s = jax.lax.dot_general(qkv[h][0], qkv[h][1], (((1,), (1,)), ((), ())),
                                    preferred_element_type=F32)
            s = jnp.where(mask, s, -1e30)
            sc[h] = (s, jnp.max(s, axis=-1, keepdims=True))

        def st_pv(h):
            s, mx = sc.pop(h)
            p = jnp.exp2((s - mx) * c_exp)
            av[h] = (_dot(p, qkv.pop(h)[2]), jnp.sum(p, axis=-1, keepdims=True))

        def st_norm(h):
            o, l = av.pop(h)
            r = pl.reciprocal(l, approx=True)
            r = r * (2.0 - l * r)
            o = o * r
            oh[h] = o[0:32].astype(BF16)
            oo[h, pl.ds(r8, 8), :] = o[32:40].astype(BF16)

        def st_out(h):
            w = jnp.concatenate([wo_s[n, h * E:(h + 1) * E, :] for n in range(NT)], axis=1)
            r = _dot(oh.pop(h), w)
            acc_o[:] = [r if not acc_o else acc_o[0] + r]

        stages = ((st_proj, 0), (st_score, 8), (st_pv, 16), (st_norm, 20), (st_out, 28))
        for t in range(H + stages[-1][1]):
            for fn, lag in stages:
                if 0 <= t - lag < H:
                    fn(t - lag)

        res = acc_o[0]
        hb[pl.ds(r0, 24), :] = hb[pl.ds(r0, 24), :] + res[8:32]
        return res[0:8]

    with jax.named_scope('S_rec'):
        jax.lax.fori_loop(0, NSEG, step, mem0_ref[...].astype(F32), unroll=REC_UNROLL)

    def tail_out(c, carry):
        r = pl.multiple_of(c * 128, 128)
        lhs = jnp.concatenate([oo[h, pl.ds(r, 128), :] for h in range(H)], axis=1)
        for n in range(NT):
            res = _dot(lhs, wo_s[n])
            cs = slice(n * 128, (n + 1) * 128)
            for s in range(16):
                rr = pl.multiple_of(c * (16 * SEG) + s * SEG + 24, 8)
                hb[pl.ds(rr, 8), cs] = hb[pl.ds(rr, 8), cs] + res[8 * s:8 * s + 8]
        return carry

    with jax.named_scope('S_tailout'):
        jax.lax.fori_loop(0, 4, tail_out, 0)

    cp_w1.wait()
    cp_w2.wait()
    cp_w3.wait()
    cp_w4.wait()
    gb[0:PAD, :] = jnp.zeros((PAD, D), BF16)
    yb = xn

    def stage1(r, n):
        y = _ln(hb[pl.ds(r, n), :])
        yb[pl.ds(r, n), :] = y
        z = _ln(y).astype(BF16)
        g = _gelu(_dot(z, w1_s[...]))
        gb[pl.ds(r + PAD, n), :] = g.astype(BF16)

    def stage2(b, wait_unused=None):
        r = pl.multiple_of(b * RB, RB)
        c = D // 4
        parts = []
        for gi, sh in enumerate((-1, 1, -2, 2)):
            win = gb[pl.ds(r, RB + 2 * PAD), gi * c:(gi + 1) * c].astype(F32)
            parts.append(win[PAD + sh:PAD + sh + RB].astype(BF16))
        gs = jnp.concatenate(parts, axis=1)
        x1 = yb[pl.ds(r, RB), :] + _dot(gs, w2_s[...])
        z2 = _ln(x1).astype(BF16)
        acc = hb[pl.ds(r, RB), :] + x1
        for f in range(FF // FC):
            a = _gelu(_dot(z2, w3_s[:, f * FC:(f + 1) * FC])).astype(BF16)
            acc = acc + _dot(a, w4_s[f * FC:(f + 1) * FC, :])
        outb[pl.ds(r, RB), :] = acc.astype(BF16)
        pltpu.make_async_copy(outb.at[pl.ds(r, RB), :], out_hbm.at[pl.ds(r, RB), :],
                              osems.at[b]).start()

    with jax.named_scope('S_pro'):
        stage1(0, RB + PAD)

    def mlp(b, carry):
        stage2(b)
        stage1(pl.multiple_of(jnp.minimum(b + 1, NRB - 1) * RB + PAD, PAD), RB)
        return carry

    with jax.named_scope('S_mlp'):
        jax.lax.fori_loop(0, NRB, mlp, 0)

    for b in range(NRB):
        pltpu.make_async_copy(outb.at[pl.ds(b * RB, RB), :], out_hbm.at[pl.ds(b * RB, RB), :],
                              osems.at[b]).wait()


@functools.partial(jax.jit, static_argnames=("A_seg_len",))
def pallas_sequential_preLN__memory_aug_recurrent_mem_tr__mixer_s_mlp__prompt_kernel(
    A_x: jax.Array,
    A_mem0: jax.Array,
    A_Wq: jax.Array,
    A_Wk: jax.Array,
    A_Wv: jax.Array,
    A_Wo: jax.Array,
    A_seg_len: int,
    B_x: jax.Array,
    B_w1: jax.Array,
    B_w2: jax.Array,
    B_w3: jax.Array,
    B_w4: jax.Array,
):
    assert A_seg_len == SEG
    assert A_x.shape == (1, S, D) and A_mem0.shape == (1, M, D) and A_Wq.shape == (D, H, E)
    any_spec = pl.BlockSpec(memory_space=pl.ANY)
    vm = pltpu.VMEM
    out = pl.pallas_call(
        _kernel,
        out_shape=jax.ShapeDtypeStruct((S, D), A_x.dtype),
        in_specs=[any_spec, any_spec, pl.BlockSpec(memory_space=pltpu.VMEM)] + [any_spec] * 8,
        out_specs=any_spec,
        scratch_shapes=[
            vm((3 * H, D // 2, E), jnp.int32),
            vm((NT, H * E, 128), BF16),
            vm((8 * (D // 4) * H, E), BF16),
            vm((H, 512, E), F32),
            vm((S + PAD, D), F32), vm((S + PAD, D), F32),
            vm((NSEG, 8, D), BF16),
            vm((4, 512, D // 4), BF16),
            vm((3 * H, 512, E), BF16),
            vm((H, 512, E), BF16),
            vm((D, D), BF16), vm((D, D), BF16), vm((D, FF), BF16), vm((FF, D), BF16),
            vm((S + 2 * PAD, D), BF16),
            vm((S, D), BF16),
            pltpu.SemaphoreType.DMA((33,)),
            pltpu.SemaphoreType.DMA((NRB,)),
        ],
        compiler_params=pltpu.CompilerParams(vmem_limit_bytes=122 * 2 ** 20),
    )(A_x.reshape(S, D), A_x.reshape(NSEG, SEG, D), A_mem0.reshape(M, D),
      A_Wq.reshape(D * H, E), A_Wk.reshape(D * H, E), A_Wv.reshape(D * H, E),
      A_Wo.reshape(H * E, D), B_w1, B_w2, B_w3, B_w4)
    return out.reshape(1, S, D)
```

```python
import functools

import jax
import jax.numpy as jnp
import numpy as np
import jax.experimental.pallas as pl
import jax.experimental.pallas.tpu as pltpu

F32 = jnp.float32
BF16 = jnp.bfloat16

S = 2048
D = 1024
H = 32
E = 128
M = 8
SEG = 32
NSEG = S // SEG
FF = 3584
NT = D // 128
EPS = 1e-5
PAD = 16
RB = 128
NRB = S // RB
FC = 896
REC_UNROLL = 2
ORDER = 1
MLP_UNROLL = 1
PROJ_UNROLL = 1
MIDF = 0


def _ln(x):
    m = jnp.mean(x, axis=-1, keepdims=True)
    c = x - m
    v = jnp.mean(c * c, axis=-1, keepdims=True)
    return c * jax.lax.rsqrt(v + EPS)


def _gelu(x):
    return jax.nn.gelu(x, approximate=True)


def _dot(a, b):
    return jnp.dot(a, b, preferred_element_type=F32)


def _kernel(x_hbm, x3_hbm, mem0_ref, wq_hbm, wk_hbm, wv_hbm, wo_hbm, w1_hbm, w2_hbm, w3_hbm, w4_hbm,
            out_hbm,
            w_s, wo_s, st, acc, xn, hb, xr, xo, qkvo, oo,
            w1_s, w2_s, w3_s, w4_s, gb, outb, sems, osems):
    NKC = 4
    DC = D // NKC
    IK, IV, IQ = 0, 1, 2

    cp_x3 = pltpu.make_async_copy(x3_hbm.at[:, pl.ds(24, 8), :], xr, sems.at[0])

    cp_x = pltpu.make_async_copy(x_hbm, gb.at[pl.ds(PAD, S), :], sems.at[1])

    def cp_w(src, m, c):
        n = DC * H
        slot = (m * NKC + c) % 8
        return pltpu.make_async_copy(src.at[pl.ds(pl.multiple_of(c * n, n), n), :],
                                     st.at[pl.ds(pl.multiple_of(slot * n, n), n), :],
                                     sems.at[9 + m * NKC + c])

    def wait_w(j):
        n = DC * H
        slot = pl.multiple_of((j % 8) * n, n)
        pltpu.make_async_copy(st.at[pl.ds(slot, n), :], st.at[pl.ds(slot, n), :],
                              sems.at[9 + j]).wait()

    cp_wo = [pltpu.make_async_copy(wo_hbm.at[:, pl.ds(n * 128, 128)], wo_s.at[n], sems.at[21 + n])
             for n in range(NT)]
    cp_w1 = pltpu.make_async_copy(w1_hbm, w1_s, sems.at[29])
    cp_w2 = pltpu.make_async_copy(w2_hbm, w2_s, sems.at[30])
    cp_w3 = pltpu.make_async_copy(w3_hbm, w3_s, sems.at[31])
    cp_w4 = pltpu.make_async_copy(w4_hbm, w4_s, sems.at[32])

    cp_x3.start()
    for c in range(NKC):
        cp_w(wk_hbm, IK, c).start()
    for c in range(NKC):
        cp_w(wv_hbm, IV, c).start()

    RP = 4

    def relayout_piece(j, p, q):
        wi = st.bitcast(jnp.int32)
        sub = wi.at[pl.ds(pl.multiple_of((j % 8) * (DC * 16), DC * 16), DC * 16), :]
        n = DC // RP
        dr = pl.multiple_of((j % NKC) * (DC // 2) + q * (n // 2), n // 2)
        hb0 = (j // NKC) * H
        w = sub[pl.ds(p + q * n * 16, n, stride=16), :]
        lo = jax.lax.bitcast_convert_type(w << 16, F32).astype(BF16)
        hi = jax.lax.bitcast_convert_type(w & np.int32(-65536), F32).astype(BF16)
        w_s[hb0 + 2 * p, pl.ds(dr, n // 2), :] = pltpu.bitcast(lo, jnp.int32)
        w_s[hb0 + 2 * p + 1, pl.ds(dr, n // 2), :] = pltpu.bitcast(hi, jnp.int32)

    def wtile(m, h):
        return pltpu.bitcast(w_s[m * H + h], BF16)

    hb[S:S + PAD, :] = jnp.zeros((PAD, D), F32)

    with jax.named_scope('S_p0'):
        cp_x3.wait()
        for g in range(4):
            y = _ln(jnp.concatenate([xr[16 * g + s].astype(F32) for s in range(16)], axis=0))
            y = y.astype(BF16)
            for kc in range(NKC):
                xo[kc, g * 128:(g + 1) * 128, :] = y[:, kc * DC:(kc + 1) * DC]
        wait_w(0)
        for p in range(H // 2):
            for q in range(RP):
                relayout_piece(0, p, q)

    def proj(j, carry):
        @pl.when(j < 11)
        def _():
            wait_w(j + 1)

        @pl.when(j < NKC)
        def _():
            cp_w(wq_hbm, IQ, j).start()

        @pl.when(j == NKC)
        def _():
            cp_x.start()
            for c in cp_wo:
                c.start()

        jn = jnp.minimum(j + 1, 11)
        kc = j % NKC
        hb0 = (j // NKC) * H
        dr = pl.multiple_of(kc * (DC // 2), DC // 2)
        first = kc == 0
        RS = 128
        items = [(h, r) for h in range(H) for r in range(0, 512, RS)]
        for t, (h, r) in enumerate(items):
            w = pltpu.bitcast(w_s[hb0 + h, pl.ds(dr, DC // 2), :], BF16)
            res = _dot(xo[kc, r:r + RS, :], w)
            if t % 2 == 1:
                relayout_piece(jn, (t // 2) // RP, (t // 2) % RP)
            new = res + jnp.where(first, 0.0, acc[h, r:r + RS, :])
            acc[h, r:r + RS, :] = new
            qkvo[hb0 + h, r:r + RS, :] = new.astype(BF16)
        return carry

    with jax.named_scope('S_proj'):
        jax.lax.fori_loop(0, 12, proj, 0, unroll=PROJ_UNROLL)

    cp_w1.start()
    cp_w2.start()
    cp_w3.start()
    cp_w4.start()
    cp_x.wait()
    xn[0:SEG, :] = _ln(gb[PAD:PAD + SEG, :].astype(F32))
    for c in cp_wo:
        c.wait()

    L = M + SEG
    c_exp = (E ** -0.5) * 1.4426950408889634

    def step(i, mem):
        r0 = pl.multiple_of(i * SEG, SEG)
        r8 = pl.multiple_of(i * 8, 8)
        lhs = jnp.concatenate([mem, xn[pl.ds(r0, 24), :]], axis=0).astype(BF16)
        row = jax.lax.broadcasted_iota(jnp.int32, (L, L), 0)
        col = jax.lax.broadcasted_iota(jnp.int32, (L, L), 1)
        mask = (row < M) | (row >= col)

        rn = pl.multiple_of(jnp.minimum(i + 1, NSEG - 1) * SEG, SEG)
        xn_next = _ln(gb[pl.ds(PAD + rn, SEG), :].astype(F32))

        qkv, sc, av, oh = {}, {}, {}, {}
        acc_o = []

        def st_proj(h):
            qkv[h] = tuple(
                jnp.concatenate([_dot(lhs, wtile(m, h)),
                                 qkvo[m * H + h, pl.ds(r8, 8), :].astype(F32)], axis=0)
                for m in (IQ, IK, IV))

        def st_score(h):
            s = jax.lax.dot_general(qkv[h][0], qkv[h][1], (((1,), (1,)), ((), ())),
                                    preferred_element_type=F32)
            s = jnp.where(mask, s, -1e30)
            sc[h] = (s, jnp.max(s, axis=-1, keepdims=True))

        def st_pv(h):
            s, mx = sc.pop(h)
            p = jnp.exp2((s - mx) * c_exp)
            av[h] = (_dot(p, qkv.pop(h)[2]), jnp.sum(p, axis=-1, keepdims=True))

        def st_norm(h):
            o, l = av.pop(h)
            r = pl.reciprocal(l, approx=True)
            r = r * (2.0 - l * r)
            o = o * r
            oh[h] = o[0:32].astype(BF16)
            oo[h, pl.ds(r8, 8), :] = o[32:40].astype(BF16)

        def st_out(h):
            w = jnp.concatenate([wo_s[n, h * E:(h + 1) * E, :] for n in range(NT)], axis=1)
            r = _dot(oh.pop(h), w)
            acc_o[:] = [r if not acc_o else acc_o[0] + r]

        stages = ((st_proj, 0), (st_score, 8), (st_pv, 16), (st_norm, 20), (st_out, 28))
        for t in range(H + stages[-1][1]):
            for fn, lag in stages:
                if 0 <= t - lag < H:
                    fn(t - lag)

        xn[pl.ds(rn, SEG), :] = xn_next
        res = acc_o[0]
        xv = gb[pl.ds(PAD + r0, SEG), :].astype(F32)
        hb[pl.ds(r0, SEG), :] = jnp.concatenate([xv[0:24] + res[8:32], xv[24:32]], axis=0)
        return res[0:8]

    with jax.named_scope('S_rec'):
        jax.lax.fori_loop(0, NSEG, step, mem0_ref[...].astype(F32), unroll=REC_UNROLL)

    def tail_out(c, carry):
        r = pl.multiple_of(c * 128, 128)
        lhs = jnp.concatenate([oo[h, pl.ds(r, 128), :] for h in range(H)], axis=1)
        for n in range(NT):
            res = _dot(lhs, wo_s[n])
            cs = slice(n * 128, (n + 1) * 128)
            for s in range(16):
                rr = pl.multiple_of(c * (16 * SEG) + s * SEG + 24, 8)
                hb[pl.ds(rr, 8), cs] = hb[pl.ds(rr, 8), cs] + res[8 * s:8 * s + 8]
        return carry

    with jax.named_scope('S_tailout'):
        jax.lax.fori_loop(0, 4, tail_out, 0)

    cp_w1.wait()
    cp_w2.wait()
    cp_w3.wait()
    cp_w4.wait()
    gb[0:PAD, :] = jnp.zeros((PAD, D), BF16)
    yb = xn

    def stage1(r, n):
        y = _ln(hb[pl.ds(r, n), :])
        yb[pl.ds(r, n), :] = y
        z = _ln(y).astype(BF16)
        g = _gelu(_dot(z, w1_s[...]))
        gb[pl.ds(r + PAD, n), :] = g.astype(BF16)

    def stage2a(b):
        r = pl.multiple_of(b * RB, RB)
        c = D // 4
        parts = []
        for gi, sh in enumerate((-1, 1, -2, 2)):
            win = gb[pl.ds(r, RB + 2 * PAD), gi * c:(gi + 1) * c].astype(F32)
            parts.append(win[PAD + sh:PAD + sh + RB].astype(BF16))
        gs = jnp.concatenate(parts, axis=1)
        return yb[pl.ds(r, RB), :] + _dot(gs, w2_s[...])

    def stage2b(b, x1, mid=None):
        r = pl.multiple_of(b * RB, RB)
        z2 = _ln(x1).astype(BF16)
        acc = hb[pl.ds(r, RB), :] + x1
        for f in range(FF // FC):
            a = _gelu(_dot(z2, w3_s[:, f * FC:(f + 1) * FC])).astype(BF16)
            if mid is not None and f == MIDF:
                mid()
            acc = acc + _dot(a, w4_s[f * FC:(f + 1) * FC, :])
        outb[pl.ds(r, RB), :] = acc.astype(BF16)
        pltpu.make_async_copy(outb.at[pl.ds(r, RB), :], out_hbm.at[pl.ds(r, RB), :],
                              osems.at[b]).start()

    with jax.named_scope('S_pro'):
        stage1(0, RB + PAD)

    def mlp(b, carry):
        s1 = lambda: stage1(pl.multiple_of(jnp.minimum(b + 1, NRB - 1) * RB + PAD, PAD), RB)
        if ORDER == 0:
            stage2b(b, stage2a(b))
            s1()
        elif ORDER == 1:
            x1 = stage2a(b)
            s1()
            stage2b(b, x1)
        elif ORDER == 2:
            stage2b(b, stage2a(b), s1)
        return carry

    with jax.named_scope('S_mlp'):
        jax.lax.fori_loop(0, NRB, mlp, 0, unroll=MLP_UNROLL)

    for b in range(NRB):
        pltpu.make_async_copy(outb.at[pl.ds(b * RB, RB), :], out_hbm.at[pl.ds(b * RB, RB), :],
                              osems.at[b]).wait()


@functools.partial(jax.jit, static_argnames=("A_seg_len",))
def pallas_sequential_preLN__memory_aug_recurrent_mem_tr__mixer_s_mlp__prompt_kernel(
    A_x: jax.Array,
    A_mem0: jax.Array,
    A_Wq: jax.Array,
    A_Wk: jax.Array,
    A_Wv: jax.Array,
    A_Wo: jax.Array,
    A_seg_len: int,
    B_x: jax.Array,
    B_w1: jax.Array,
    B_w2: jax.Array,
    B_w3: jax.Array,
    B_w4: jax.Array,
):
    assert A_seg_len == SEG
    assert A_x.shape == (1, S, D) and A_mem0.shape == (1, M, D) and A_Wq.shape == (D, H, E)
    any_spec = pl.BlockSpec(memory_space=pl.ANY)
    vm = pltpu.VMEM
    out = pl.pallas_call(
        _kernel,
        out_shape=jax.ShapeDtypeStruct((S, D), A_x.dtype),
        in_specs=[any_spec, any_spec, pl.BlockSpec(memory_space=pltpu.VMEM)] + [any_spec] * 8,
        out_specs=any_spec,
        scratch_shapes=[
            vm((3 * H, D // 2, E), jnp.int32),
            vm((NT, H * E, 128), BF16),
            vm((8 * (D // 4) * H, E), BF16),
            vm((H, 512, E), F32),
            vm((S + PAD, D), F32), vm((S + PAD, D), F32),
            vm((NSEG, 8, D), BF16),
            vm((4, 512, D // 4), BF16),
            vm((3 * H, 512, E), BF16),
            vm((H, 512, E), BF16),
            vm((D, D), BF16), vm((D, D), BF16), vm((D, FF), BF16), vm((FF, D), BF16),
            vm((S + 2 * PAD, D), BF16),
            vm((S, D), BF16),
            pltpu.SemaphoreType.DMA((33,)),
            pltpu.SemaphoreType.DMA((NRB,)),
        ],
        compiler_params=pltpu.CompilerParams(vmem_limit_bytes=122 * 2 ** 20),
    )(A_x.reshape(S, D), A_x.reshape(NSEG, SEG, D), A_mem0.reshape(M, D),
      A_Wq.reshape(D * H, E), A_Wk.reshape(D * H, E), A_Wv.reshape(D * H, E),
      A_Wo.reshape(H * E, D), B_w1, B_w2, B_w3, B_w4)
    return out.reshape(1, S, D)
```

```python
import functools

import jax
import jax.numpy as jnp
import numpy as np
import jax.experimental.pallas as pl
import jax.experimental.pallas.tpu as pltpu

F32 = jnp.float32
BF16 = jnp.bfloat16

S = 2048
D = 1024
H = 32
E = 128
M = 8
SEG = 32
NSEG = S // SEG
FF = 3584
NT = D // 128
EPS = 1e-5
PAD = 16
RB = 128
NRB = S // RB
FC = 896
REC_UNROLL = 2
ORDER = 1
MLP_UNROLL = 1
PEEL_PROJ = 1
PEEL_MLP = 0
PROJ_UNROLL = 1
MIDF = 0


def _ln(x):
    m = jnp.mean(x, axis=-1, keepdims=True)
    c = x - m
    v = jnp.mean(c * c, axis=-1, keepdims=True)
    return c * jax.lax.rsqrt(v + EPS)


def _gelu(x):
    return jax.nn.gelu(x, approximate=True)


def _dot(a, b):
    return jnp.dot(a, b, preferred_element_type=F32)


def _kernel(x_hbm, x3_hbm, mem0_ref, wq_hbm, wk_hbm, wv_hbm, wo_hbm, w1_hbm, w2_hbm, w3_hbm, w4_hbm,
            out_hbm,
            w_s, wo_s, st, acc, xn, hb, xr, xo, qkvo, oo,
            w1_s, w2_s, w3_s, w4_s, gb, outb, sems, osems):
    NKC = 4
    DC = D // NKC
    IK, IV, IQ = 0, 1, 2

    cp_x3 = pltpu.make_async_copy(x3_hbm.at[:, pl.ds(24, 8), :], xr, sems.at[0])

    RP = 4
    NC = DC * H
    NP = NC // RP
    WB = 16

    def cp_w(src, m, c):
        slot = (m * NKC + c) % 8
        return pltpu.make_async_copy(src.at[pl.ds(pl.multiple_of(c * NC, NC), NC), :],
                                     st.at[pl.ds(pl.multiple_of(slot * NC, NC), NC), :],
                                     sems.at[WB + m * NKC + c])

    cp_w0 = [pltpu.make_async_copy(wk_hbm.at[pl.ds(q * NP, NP), :], st.at[pl.ds(q * NP, NP), :],
                                   sems.at[WB + 13 + q]) for q in range(RP)]

    def wait_w(j):
        r = pl.multiple_of((j % 8) * NC, NC)
        pltpu.make_async_copy(st.at[pl.ds(r, NC), :], st.at[pl.ds(r, NC), :],
                              sems.at[WB + j]).wait()

    XA = NC * E // D
    cp_xa = pltpu.make_async_copy(x_hbm.at[pl.ds(0, XA), :], gb.at[pl.ds(PAD, XA), :],
                                  sems.at[WB + 12])
    cp_xb = pltpu.make_async_copy(x_hbm.at[pl.ds(XA, S - XA), :],
                                  gb.at[pl.ds(PAD + XA, S - XA), :], sems.at[1])

    cp_wo = [pltpu.make_async_copy(wo_hbm.at[:, pl.ds(n * 128, 128)], wo_s.at[n], sems.at[2 + n])
             for n in range(NT)]
    cp_w1 = pltpu.make_async_copy(w1_hbm, w1_s, sems.at[10])
    cp_w2 = pltpu.make_async_copy(w2_hbm, w2_s, sems.at[11])
    cp_w3 = pltpu.make_async_copy(w3_hbm, w3_s, sems.at[12])
    cp_w4 = pltpu.make_async_copy(w4_hbm, w4_s, sems.at[13])

    cp_x3.start()
    for c in cp_w0:
        c.start()
    for c in range(1, NKC):
        cp_w(wk_hbm, IK, c).start()
    for c in range(NKC):
        cp_w(wv_hbm, IV, c).start()

    def relayout_piece(j, p, q):
        wi = st.bitcast(jnp.int32)
        sub = wi.at[pl.ds(pl.multiple_of((j % 8) * (DC * 16), DC * 16), DC * 16), :]
        n = DC // RP
        dr = pl.multiple_of((j % NKC) * (DC // 2) + q * (n // 2), n // 2)
        hb0 = (j // NKC) * H
        w = sub[pl.ds(p + q * n * 16, n, stride=16), :]
        lo = jax.lax.bitcast_convert_type(w << 16, F32).astype(BF16)
        hi = jax.lax.bitcast_convert_type(w & np.int32(-65536), F32).astype(BF16)
        w_s[hb0 + 2 * p, pl.ds(dr, n // 2), :] = pltpu.bitcast(lo, jnp.int32)
        w_s[hb0 + 2 * p + 1, pl.ds(dr, n // 2), :] = pltpu.bitcast(hi, jnp.int32)

    def wtile(m, h):
        return pltpu.bitcast(w_s[m * H + h], BF16)

    hb[S:S + PAD, :] = jnp.zeros((PAD, D), F32)

    with jax.named_scope('S_p0'):
        cp_x3.wait()
        for g in range(4):
            y = _ln(jnp.concatenate([xr[16 * g + s].astype(F32) for s in range(16)], axis=0))
            y = y.astype(BF16)
            for kc in range(NKC):
                xo[kc, g * 128:(g + 1) * 128, :] = y[:, kc * DC:(kc + 1) * DC]
        for q in range(RP):
            cp_w0[q].wait()
            for p in range(H // 2):
                relayout_piece(0, p, q)

    RS = 128
    items = [(h, r) for h in range(H) for r in range(0, 512, RS)]

    def proj_first():
        cp_w(wq_hbm, IQ, 0).start()
        for t, (h, r) in enumerate(items):
            w = pltpu.bitcast(w_s[h, 0:DC // 2, :], BF16)
            res = _dot(xo[0, r:r + RS, :], w)
            if t == len(items) // 2:
                wait_w(1)
            if t >= len(items) // 2:
                p, q = divmod(t - len(items) // 2, RP)
                relayout_piece(1, p, q)
            acc[h, r:r + RS, :] = res

    def proj(j, carry):
        @pl.when(j < NKC)
        def _():
            cp_w(wq_hbm, IQ, j).start()

        @pl.when(j == NKC)
        def _():
            cp_xa.start()
            cp_xb.start()
            for c in cp_wo:
                c.start()

        wait_w(j + 1)
        jn = jnp.minimum(j + 1, 11)
        kc = j % NKC
        hb0 = (j // NKC) * H
        dr = pl.multiple_of(kc * (DC // 2), DC // 2)
        first = kc == 0
        for t, (h, r) in enumerate(items):
            w = pltpu.bitcast(w_s[hb0 + h, pl.ds(dr, DC // 2), :], BF16)
            res = _dot(xo[kc, r:r + RS, :], w)
            if t % 2 == 1:
                p, q = divmod(t // 2, RP)
                relayout_piece(jn, p, q)
            new = res + jnp.where(first, 0.0, acc[h, r:r + RS, :])
            acc[h, r:r + RS, :] = new
            qkvo[hb0 + h, r:r + RS, :] = new.astype(BF16)
        return carry

    with jax.named_scope('S_proj'):
        if PEEL_PROJ:
            proj_first()
        jax.lax.fori_loop(PEEL_PROJ, 12, proj, 0, unroll=PROJ_UNROLL)

    cp_w1.start()
    cp_w2.start()
    cp_w3.start()
    cp_w4.start()
    cp_xb.wait()
    xn[0:24, :] = _ln(gb[PAD:PAD + SEG, :].astype(F32)[0:24])
    for c in cp_wo:
        c.wait()

    L = M + SEG
    c_exp = (E ** -0.5) * 1.4426950408889634

    def step(i, mem):
        r0 = pl.multiple_of(i * SEG, SEG)
        r8 = pl.multiple_of(i * 8, 8)
        lhs = jnp.concatenate([mem, xn[pl.ds(r0, 24), :]], axis=0).astype(BF16)
        row = jax.lax.broadcasted_iota(jnp.int32, (L, L), 0)
        col = jax.lax.broadcasted_iota(jnp.int32, (L, L), 1)
        mask = (row < M) | (row >= col)

        rn = pl.multiple_of(jnp.minimum(i + 1, NSEG - 1) * SEG, SEG)
        xn_next = _ln(gb[pl.ds(PAD + rn, SEG), :].astype(F32)[0:24])

        qkv, sc, av, oh = {}, {}, {}, {}
        acc_o = []

        def st_proj(h):
            qkv[h] = tuple(
                jnp.concatenate([_dot(lhs, wtile(m, h)),
                                 qkvo[m * H + h, pl.ds(r8, 8), :].astype(F32)], axis=0)
                for m in (IQ, IK, IV))

        def st_score(h):
            s = jax.lax.dot_general(qkv[h][0], qkv[h][1], (((1,), (1,)), ((), ())),
                                    preferred_element_type=F32)
            s = jnp.where(mask, s, -1e30)
            sc[h] = (s, jnp.max(s, axis=-1, keepdims=True))

        def st_pv(h):
            s, mx = sc.pop(h)
            p = jnp.exp2((s - mx) * c_exp)
            av[h] = (_dot(p, qkv.pop(h)[2]), jnp.sum(p, axis=-1, keepdims=True))

        def st_norm(h):
            o, l = av.pop(h)
            r = pl.reciprocal(l, approx=True)
            r = r * (2.0 - l * r)
            o = o * r
            oh[h] = o[0:32].astype(BF16)
            oo[h, pl.ds(r8, 8), :] = o[32:40].astype(BF16)

        def st_out(h):
            w = jnp.concatenate([wo_s[n, h * E:(h + 1) * E, :] for n in range(NT)], axis=1)
            r = _dot(oh.pop(h), w)
            acc_o[:] = [r if not acc_o else acc_o[0] + r]

        stages = ((st_proj, 0), (st_score, 8), (st_pv, 16), (st_norm, 20), (st_out, 28))
        for t in range(H + stages[-1][1]):
            for fn, lag in stages:
                if 0 <= t - lag < H:
                    fn(t - lag)

        xn[pl.ds(rn, 24), :] = xn_next
        res = acc_o[0]
        xv = gb[pl.ds(PAD + r0, SEG), :].astype(F32)
        hb[pl.ds(r0, SEG), :] = jnp.concatenate([xv[0:24] + res[8:32], xv[24:32]], axis=0)
        return res[0:8]

    with jax.named_scope('S_rec'):
        jax.lax.fori_loop(0, NSEG, step, mem0_ref[...].astype(F32), unroll=REC_UNROLL)

    def tail_out(c, carry):
        r = pl.multiple_of(c * 128, 128)
        lhs = jnp.concatenate([oo[h, pl.ds(r, 128), :] for h in range(H)], axis=1)
        for n in range(NT):
            res = _dot(lhs, wo_s[n])
            cs = slice(n * 128, (n + 1) * 128)
            for s in range(16):
                rr = pl.multiple_of(c * (16 * SEG) + s * SEG + 24, 8)
                hb[pl.ds(rr, 8), cs] = hb[pl.ds(rr, 8), cs] + res[8 * s:8 * s + 8]
        return carry

    with jax.named_scope('S_tailout'):
        jax.lax.fori_loop(0, 4, tail_out, 0)

    cp_w1.wait()
    cp_w2.wait()
    cp_w3.wait()
    cp_w4.wait()
    gb[0:PAD, :] = jnp.zeros((PAD, D), BF16)
    yb = xn

    def stage1(r, n):
        y = _ln(hb[pl.ds(r, n), :])
        yb[pl.ds(r, n), :] = y
        z = _ln(y).astype(BF16)
        g = _gelu(_dot(z, w1_s[...]))
        gb[pl.ds(r + PAD, n), :] = g.astype(BF16)

    def stage2a(b):
        r = b * RB if isinstance(b, int) else pl.multiple_of(b * RB, RB)
        c = D // 4
        parts = []
        for gi, sh in enumerate((-1, 1, -2, 2)):
            win = gb[pl.ds(r, RB + 2 * PAD), gi * c:(gi + 1) * c].astype(F32)
            parts.append(win[PAD + sh:PAD + sh + RB].astype(BF16))
        gs = jnp.concatenate(parts, axis=1)
        return yb[pl.ds(r, RB), :] + _dot(gs, w2_s[...])

    def stage2b(b, x1, mid=None):
        r = b * RB if isinstance(b, int) else pl.multiple_of(b * RB, RB)
        z2 = _ln(x1).astype(BF16)
        acc = hb[pl.ds(r, RB), :] + x1
        for f in range(FF // FC):
            a = _gelu(_dot(z2, w3_s[:, f * FC:(f + 1) * FC])).astype(BF16)
            if mid is not None and f == MIDF:
                mid()
            acc = acc + _dot(a, w4_s[f * FC:(f + 1) * FC, :])
        outb[pl.ds(r, RB), :] = acc.astype(BF16)
        pltpu.make_async_copy(outb.at[pl.ds(r, RB), :], out_hbm.at[pl.ds(r, RB), :],
                              osems.at[b]).start()

    with jax.named_scope('S_pro'):
        stage1(0, RB + PAD)

    def mlp(b, carry):
        s1 = lambda: stage1(pl.multiple_of(jnp.minimum(b + 1, NRB - 1) * RB + PAD, PAD), RB)
        if ORDER == 0:
            stage2b(b, stage2a(b))
            s1()
        elif ORDER == 1:
            x1 = stage2a(b)
            s1()
            stage2b(b, x1)
        elif ORDER == 2:
            stage2b(b, stage2a(b), s1)
        return carry

    with jax.named_scope('S_mlp'):
        jax.lax.fori_loop(0, NRB - PEEL_MLP, mlp, 0, unroll=MLP_UNROLL)
        if PEEL_MLP:
            stage2b(NRB - 1, stage2a(NRB - 1))

    for b in range(NRB):
        pltpu.make_async_copy(outb.at[pl.ds(b * RB, RB), :], out_hbm.at[pl.ds(b * RB, RB), :],
                              osems.at[b]).wait()


@functools.partial(jax.jit, static_argnames=("A_seg_len",))
def pallas_sequential_preLN__memory_aug_recurrent_mem_tr__mixer_s_mlp__prompt_kernel(
    A_x: jax.Array,
    A_mem0: jax.Array,
    A_Wq: jax.Array,
    A_Wk: jax.Array,
    A_Wv: jax.Array,
    A_Wo: jax.Array,
    A_seg_len: int,
    B_x: jax.Array,
    B_w1: jax.Array,
    B_w2: jax.Array,
    B_w3: jax.Array,
    B_w4: jax.Array,
):
    assert A_seg_len == SEG
    assert A_x.shape == (1, S, D) and A_mem0.shape == (1, M, D) and A_Wq.shape == (D, H, E)
    any_spec = pl.BlockSpec(memory_space=pl.ANY)
    vm = pltpu.VMEM
    out = pl.pallas_call(
        _kernel,
        out_shape=jax.ShapeDtypeStruct((S, D), A_x.dtype),
        in_specs=[any_spec, any_spec, pl.BlockSpec(memory_space=pltpu.VMEM)] + [any_spec] * 8,
        out_specs=any_spec,
        scratch_shapes=[
            vm((3 * H, D // 2, E), jnp.int32),
            vm((NT, H * E, 128), BF16),
            vm((8 * (D // 4) * H, E), BF16),
            vm((H, 512, E), F32),
            vm((S + PAD, D), F32), vm((S + PAD, D), F32),
            vm((NSEG, 8, D), BF16),
            vm((4, 512, D // 4), BF16),
            vm((3 * H, 512, E), BF16),
            vm((H, 512, E), BF16),
            vm((D, D), BF16), vm((D, D), BF16), vm((D, FF), BF16), vm((FF, D), BF16),
            vm((S + 2 * PAD, D), BF16),
            vm((S, D), BF16),
            pltpu.SemaphoreType.DMA((16 + 13 + 4,)),
            pltpu.SemaphoreType.DMA((NRB,)),
        ],
        compiler_params=pltpu.CompilerParams(vmem_limit_bytes=122 * 2 ** 20),
    )(A_x.reshape(S, D), A_x.reshape(NSEG, SEG, D), A_mem0.reshape(M, D),
      A_Wq.reshape(D * H, E), A_Wk.reshape(D * H, E), A_Wv.reshape(D * H, E),
      A_Wo.reshape(H * E, D), B_w1, B_w2, B_w3, B_w4)
    return out.reshape(1, S, D)
```

```python
import functools

import jax
import jax.numpy as jnp
import numpy as np
import jax.experimental.pallas as pl
import jax.experimental.pallas.tpu as pltpu

F32 = jnp.float32
BF16 = jnp.bfloat16

S = 2048
D = 1024
H = 32
E = 128
M = 8
SEG = 32
NSEG = S // SEG
FF = 3584
NT = D // 128
EPS = 1e-5
PAD = 16
RB = 128
NRB = S // RB
FC = 896
REC_UNROLL = 2
ORDER = 1
MLP_UNROLL = 1
PEEL_PROJ = 1
PEEL_MLP = 0
PROJ_UNROLL = 1
MIDF = 0


def _ln(x):
    m = jnp.mean(x, axis=-1, keepdims=True)
    c = x - m
    v = jnp.mean(c * c, axis=-1, keepdims=True)
    return c * jax.lax.rsqrt(v + EPS)


def _gelu(x):
    return jax.nn.gelu(x, approximate=True)


def _dot(a, b):
    return jnp.dot(a, b, preferred_element_type=F32)


def _kernel(x_hbm, x3_hbm, mem0_ref, wq_hbm, wk_hbm, wv_hbm, wo_hbm, w1_hbm, w2_hbm, w3_hbm, w4_hbm,
            out_hbm,
            w_s, wo_s, st, acc, xn, hb, xr, xo, qkvo, oo,
            w1_s, w2_s, w3_s, w4_s, gb, outb, sems, osems):
    NKC = 4
    DC = D // NKC
    IK, IV, IQ = 0, 1, 2

    cp_x3 = pltpu.make_async_copy(x3_hbm.at[:, pl.ds(24, 8), :], xr, sems.at[0])

    RP = 4
    NC = DC * H
    NP = NC // RP
    WB = 16

    def cp_w(src, m, c):
        slot = (m * NKC + c) % 8
        return pltpu.make_async_copy(src.at[pl.ds(pl.multiple_of(c * NC, NC), NC), :],
                                     st.at[pl.ds(pl.multiple_of(slot * NC, NC), NC), :],
                                     sems.at[WB + m * NKC + c])

    cp_w0 = [pltpu.make_async_copy(wk_hbm.at[pl.ds(q * NP, NP), :], st.at[pl.ds(q * NP, NP), :],
                                   sems.at[WB + 13 + q]) for q in range(RP)]

    def wait_w(j):
        r = pl.multiple_of((j % 8) * NC, NC)
        pltpu.make_async_copy(st.at[pl.ds(r, NC), :], st.at[pl.ds(r, NC), :],
                              sems.at[WB + j]).wait()

    cp_x = pltpu.make_async_copy(x_hbm, gb.at[pl.ds(PAD, S), :], sems.at[1])

    cp_wo = [pltpu.make_async_copy(wo_hbm.at[:, pl.ds(n * 128, 128)], wo_s.at[n], sems.at[2 + n])
             for n in range(NT)]
    cp_w1 = pltpu.make_async_copy(w1_hbm, w1_s, sems.at[10])
    cp_w2 = pltpu.make_async_copy(w2_hbm, w2_s, sems.at[11])
    cp_w3 = pltpu.make_async_copy(w3_hbm, w3_s, sems.at[12])
    cp_w4 = pltpu.make_async_copy(w4_hbm, w4_s, sems.at[13])

    cp_x3.start()
    for c in cp_w0:
        c.start()
    for c in range(1, NKC):
        cp_w(wk_hbm, IK, c).start()
    for c in range(NKC):
        cp_w(wv_hbm, IV, c).start()

    def relayout_piece(j, p, q):
        wi = st.bitcast(jnp.int32)
        sub = wi.at[pl.ds(pl.multiple_of((j % 8) * (DC * 16), DC * 16), DC * 16), :]
        n = DC // RP
        dr = pl.multiple_of((j % NKC) * (DC // 2) + q * (n // 2), n // 2)
        hb0 = (j // NKC) * H
        w = sub[pl.ds(p + q * n * 16, n, stride=16), :]
        lo = jax.lax.bitcast_convert_type(w << 16, F32).astype(BF16)
        hi = jax.lax.bitcast_convert_type(w & np.int32(-65536), F32).astype(BF16)
        w_s[hb0 + 2 * p, pl.ds(dr, n // 2), :] = pltpu.bitcast(lo, jnp.int32)
        w_s[hb0 + 2 * p + 1, pl.ds(dr, n // 2), :] = pltpu.bitcast(hi, jnp.int32)

    def wtile(m, h):
        return pltpu.bitcast(w_s[m * H + h], BF16)

    hb[S:S + PAD, :] = jnp.zeros((PAD, D), F32)

    with jax.named_scope('S_p0'):
        cp_x3.wait()
        for g in range(4):
            y = _ln(jnp.concatenate([xr[16 * g + s].astype(F32) for s in range(16)], axis=0))
            y = y.astype(BF16)
            for kc in range(NKC):
                xo[kc, g * 128:(g + 1) * 128, :] = y[:, kc * DC:(kc + 1) * DC]
        for q in range(RP):
            cp_w0[q].wait()
            for p in range(H // 2):
                relayout_piece(0, p, q)

    RS = 128
    items = [(h, r) for h in range(H) for r in range(0, 512, RS)]

    def proj_first():
        cp_w(wq_hbm, IQ, 0).start()
        for t, (h, r) in enumerate(items):
            w = pltpu.bitcast(w_s[h, 0:DC // 2, :], BF16)
            res = _dot(xo[0, r:r + RS, :], w)
            if t == len(items) // 2:
                wait_w(1)
            if t >= len(items) // 2:
                p, q = divmod(t - len(items) // 2, RP)
                relayout_piece(1, p, q)
            acc[h, r:r + RS, :] = res

    def proj(j, carry):
        @pl.when(j < NKC)
        def _():
            cp_w(wq_hbm, IQ, j).start()

        @pl.when(j == NKC)
        def _():
            cp_x.start()
            for c in cp_wo:
                c.start()

        @pl.when(j < 11)
        def _():
            wait_w(j + 1)

        jn = jnp.minimum(j + 1, 11)
        kc = j % NKC
        hb0 = (j // NKC) * H
        dr = pl.multiple_of(kc * (DC // 2), DC // 2)
        first = kc == 0
        for t, (h, r) in enumerate(items):
            w = pltpu.bitcast(w_s[hb0 + h, pl.ds(dr, DC // 2), :], BF16)
            res = _dot(xo[kc, r:r + RS, :], w)
            if t % 2 == 1:
                p, q = divmod(t // 2, RP)
                relayout_piece(jn, p, q)
            new = res + jnp.where(first, 0.0, acc[h, r:r + RS, :])
            acc[h, r:r + RS, :] = new
            qkvo[hb0 + h, r:r + RS, :] = new.astype(BF16)
        return carry

    with jax.named_scope('S_proj'):
        if PEEL_PROJ:
            proj_first()
        jax.lax.fori_loop(PEEL_PROJ, 12, proj, 0, unroll=PROJ_UNROLL)

    cp_w1.start()
    cp_w2.start()
    cp_w3.start()
    cp_w4.start()
    cp_x.wait()
    xn[0:24, :] = _ln(gb[PAD:PAD + SEG, :].astype(F32)[0:24])
    for c in cp_wo:
        c.wait()

    L = M + SEG
    c_exp = (E ** -0.5) * 1.4426950408889634

    def step(i, mem):
        r0 = pl.multiple_of(i * SEG, SEG)
        r8 = pl.multiple_of(i * 8, 8)
        lhs = jnp.concatenate([mem, xn[pl.ds(r0, 24), :]], axis=0).astype(BF16)
        row = jax.lax.broadcasted_iota(jnp.int32, (L, L), 0)
        col = jax.lax.broadcasted_iota(jnp.int32, (L, L), 1)
        mask = (row < M) | (row >= col)

        rn = pl.multiple_of(jnp.minimum(i + 1, NSEG - 1) * SEG, SEG)
        xn_next = _ln(gb[pl.ds(PAD + rn, SEG), :].astype(F32)[0:24])

        qkv, sc, av, oh = {}, {}, {}, {}
        acc_o = []

        def st_proj(h):
            qkv[h] = tuple(
                jnp.concatenate([_dot(lhs, wtile(m, h)),
                                 qkvo[m * H + h, pl.ds(r8, 8), :].astype(F32)], axis=0)
                for m in (IQ, IK, IV))

        def st_score(h):
            s = jax.lax.dot_general(qkv[h][0], qkv[h][1], (((1,), (1,)), ((), ())),
                                    preferred_element_type=F32)
            s = jnp.where(mask, s, -1e30)
            sc[h] = (s, jnp.max(s, axis=-1, keepdims=True))

        def st_pv(h):
            s, mx = sc.pop(h)
            p = jnp.exp2((s - mx) * c_exp)
            av[h] = (_dot(p, qkv.pop(h)[2]), jnp.sum(p, axis=-1, keepdims=True))

        def st_norm(h):
            o, l = av.pop(h)
            r = pl.reciprocal(l, approx=True)
            r = r * (2.0 - l * r)
            o = o * r
            oh[h] = o[0:32].astype(BF16)
            oo[h, pl.ds(r8, 8), :] = o[32:40].astype(BF16)

        def st_out(h):
            w = jnp.concatenate([wo_s[n, h * E:(h + 1) * E, :] for n in range(NT)], axis=1)
            r = _dot(oh.pop(h), w)
            acc_o[:] = [r if not acc_o else acc_o[0] + r]

        stages = ((st_proj, 0), (st_score, 8), (st_pv, 16), (st_norm, 20), (st_out, 28))
        for t in range(H + stages[-1][1]):
            for fn, lag in stages:
                if 0 <= t - lag < H:
                    fn(t - lag)

        xn[pl.ds(rn, 24), :] = xn_next
        res = acc_o[0]
        xv = gb[pl.ds(PAD + r0, SEG), :].astype(F32)
        hb[pl.ds(r0, SEG), :] = jnp.concatenate([xv[0:24] + res[8:32], xv[24:32]], axis=0)
        return res[0:8]

    with jax.named_scope('S_rec'):
        jax.lax.fori_loop(0, NSEG, step, mem0_ref[...].astype(F32), unroll=REC_UNROLL)

    def tail_out(c, carry):
        r = pl.multiple_of(c * 128, 128)
        lhs = jnp.concatenate([oo[h, pl.ds(r, 128), :] for h in range(H)], axis=1)
        for n in range(NT):
            res = _dot(lhs, wo_s[n])
            cs = slice(n * 128, (n + 1) * 128)
            for s in range(16):
                rr = pl.multiple_of(c * (16 * SEG) + s * SEG + 24, 8)
                hb[pl.ds(rr, 8), cs] = hb[pl.ds(rr, 8), cs] + res[8 * s:8 * s + 8]
        return carry

    with jax.named_scope('S_tailout'):
        jax.lax.fori_loop(0, 4, tail_out, 0)

    cp_w1.wait()
    cp_w2.wait()
    cp_w3.wait()
    cp_w4.wait()
    gb[0:PAD, :] = jnp.zeros((PAD, D), BF16)
    yb = xn

    def stage1(r, n):
        y = _ln(hb[pl.ds(r, n), :])
        yb[pl.ds(r, n), :] = y
        z = _ln(y).astype(BF16)
        g = _gelu(_dot(z, w1_s[...]))
        gb[pl.ds(r + PAD, n), :] = g.astype(BF16)

    def stage2a(b):
        r = b * RB if isinstance(b, int) else pl.multiple_of(b * RB, RB)
        c = D // 4
        parts = []
        for gi, sh in enumerate((-1, 1, -2, 2)):
            win = gb[pl.ds(r, RB + 2 * PAD), gi * c:(gi + 1) * c].astype(F32)
            parts.append(win[PAD + sh:PAD + sh + RB].astype(BF16))
        gs = jnp.concatenate(parts, axis=1)
        return yb[pl.ds(r, RB), :] + _dot(gs, w2_s[...])

    def stage2b(b, x1, mid=None):
        r = b * RB if isinstance(b, int) else pl.multiple_of(b * RB, RB)
        z2 = _ln(x1).astype(BF16)
        acc = hb[pl.ds(r, RB), :] + x1
        for f in range(FF // FC):
            a = _gelu(_dot(z2, w3_s[:, f * FC:(f + 1) * FC])).astype(BF16)
            if mid is not None and f == MIDF:
                mid()
            acc = acc + _dot(a, w4_s[f * FC:(f + 1) * FC, :])
        outb[pl.ds(r, RB), :] = acc.astype(BF16)
        pltpu.make_async_copy(outb.at[pl.ds(r, RB), :], out_hbm.at[pl.ds(r, RB), :],
                              osems.at[b]).start()

    with jax.named_scope('S_pro'):
        stage1(0, RB + PAD)

    def mlp(b, carry):
        s1 = lambda: stage1(pl.multiple_of(jnp.minimum(b + 1, NRB - 1) * RB + PAD, PAD), RB)
        if ORDER == 0:
            stage2b(b, stage2a(b))
            s1()
        elif ORDER == 1:
            x1 = stage2a(b)
            s1()
            stage2b(b, x1)
        elif ORDER == 2:
            stage2b(b, stage2a(b), s1)
        return carry

    with jax.named_scope('S_mlp'):
        jax.lax.fori_loop(0, NRB - PEEL_MLP, mlp, 0, unroll=MLP_UNROLL)
        if PEEL_MLP:
            stage2b(NRB - 1, stage2a(NRB - 1))

    for b in range(NRB):
        pltpu.make_async_copy(outb.at[pl.ds(b * RB, RB), :], out_hbm.at[pl.ds(b * RB, RB), :],
                              osems.at[b]).wait()


@functools.partial(jax.jit, static_argnames=("A_seg_len",))
def pallas_sequential_preLN__memory_aug_recurrent_mem_tr__mixer_s_mlp__prompt_kernel(
    A_x: jax.Array,
    A_mem0: jax.Array,
    A_Wq: jax.Array,
    A_Wk: jax.Array,
    A_Wv: jax.Array,
    A_Wo: jax.Array,
    A_seg_len: int,
    B_x: jax.Array,
    B_w1: jax.Array,
    B_w2: jax.Array,
    B_w3: jax.Array,
    B_w4: jax.Array,
):
    assert A_seg_len == SEG
    assert A_x.shape == (1, S, D) and A_mem0.shape == (1, M, D) and A_Wq.shape == (D, H, E)
    any_spec = pl.BlockSpec(memory_space=pl.ANY)
    vm = pltpu.VMEM
    out = pl.pallas_call(
        _kernel,
        out_shape=jax.ShapeDtypeStruct((S, D), A_x.dtype),
        in_specs=[any_spec, any_spec, pl.BlockSpec(memory_space=pltpu.VMEM)] + [any_spec] * 8,
        out_specs=any_spec,
        scratch_shapes=[
            vm((3 * H, D // 2, E), jnp.int32),
            vm((NT, H * E, 128), BF16),
            vm((8 * (D // 4) * H, E), BF16),
            vm((H, 512, E), F32),
            vm((S + PAD, D), F32), vm((S + PAD, D), F32),
            vm((NSEG, 8, D), BF16),
            vm((4, 512, D // 4), BF16),
            vm((3 * H, 512, E), BF16),
            vm((H, 512, E), BF16),
            vm((D, D), BF16), vm((D, D), BF16), vm((D, FF), BF16), vm((FF, D), BF16),
            vm((S + 2 * PAD, D), BF16),
            vm((S, D), BF16),
            pltpu.SemaphoreType.DMA((16 + 13 + 4,)),
            pltpu.SemaphoreType.DMA((NRB,)),
        ],
        compiler_params=pltpu.CompilerParams(vmem_limit_bytes=122 * 2 ** 20),
    )(A_x.reshape(S, D), A_x.reshape(NSEG, SEG, D), A_mem0.reshape(M, D),
      A_Wq.reshape(D * H, E), A_Wk.reshape(D * H, E), A_Wv.reshape(D * H, E),
      A_Wo.reshape(H * E, D), B_w1, B_w2, B_w3, B_w4)
    return out.reshape(1, S, D)
```

```python
import functools

import jax
import jax.numpy as jnp
import numpy as np
import jax.experimental.pallas as pl
import jax.experimental.pallas.tpu as pltpu

F32 = jnp.float32
BF16 = jnp.bfloat16

S = 2048
D = 1024
H = 32
E = 128
M = 8
SEG = 32
NSEG = S // SEG
FF = 3584
NT = D // 128
EPS = 1e-5
PAD = 16
RB = 128
NRB = S // RB
FC = 896
REC_UNROLL = 2
LAGS = (0, 8, 16, 20, 28)
ORDER = 1
PEEL_PROJ = 1
PROJ_UNROLL = 1
OC = 256
HS = 512
HALF = 1
T0A = 64
T0B = 64


def _ln(x):
    m = jnp.mean(x, axis=-1, keepdims=True)
    c = x - m
    v = jnp.mean(c * c, axis=-1, keepdims=True)
    return c * jax.lax.rsqrt(v + EPS)


def _gelu(x):
    return jax.nn.gelu(x, approximate=True)


def _dot(a, b):
    return jnp.dot(a, b, preferred_element_type=F32)


def _kernel(x_hbm, x3_hbm, mem0_ref, wq_hbm, wk_hbm, wv_hbm, wo_hbm, w1_hbm, w2_hbm, w3_hbm, w4_hbm,
            out_hbm,
            w_s, wo_s, st, acc, xn, hb, xr, xo, qkvo, oo,
            w1_s, w2_s, w3_s, w4_s, gb, outb, sems, osems):
    NKC = 4
    DC = D // NKC
    IK, IV, IQ = 0, 1, 2

    cp_x3 = pltpu.make_async_copy(x3_hbm.at[:, pl.ds(24, 8), :], xr, sems.at[0])

    RP = 4
    NC = DC * H
    NP = NC // RP
    WB = 16

    def cp_w(src, m, c):
        slot = (m * NKC + c) % 8
        return pltpu.make_async_copy(src.at[pl.ds(pl.multiple_of(c * NC, NC), NC), :],
                                     st.at[pl.ds(pl.multiple_of(slot * NC, NC), NC), :],
                                     sems.at[WB + m * NKC + c])

    cp_w0 = [pltpu.make_async_copy(wk_hbm.at[pl.ds(q * NP, NP), :], st.at[pl.ds(q * NP, NP), :],
                                   sems.at[WB + 13 + q]) for q in range(RP)]

    def wait_w(j):
        r = pl.multiple_of((j % 8) * NC, NC)
        pltpu.make_async_copy(st.at[pl.ds(r, NC), :], st.at[pl.ds(r, NC), :],
                              sems.at[WB + j]).wait()

    cp_x = pltpu.make_async_copy(x_hbm, gb.at[pl.ds(PAD, S), :], sems.at[1])

    cp_wo = [pltpu.make_async_copy(wo_hbm.at[:, pl.ds(n * 128, 128)], wo_s.at[n], sems.at[2 + n])
             for n in range(NT)]
    cp_w1 = pltpu.make_async_copy(w1_hbm, w1_s, sems.at[10])
    cp_w2 = pltpu.make_async_copy(w2_hbm, w2_s, sems.at[11])
    cp_w3 = pltpu.make_async_copy(w3_hbm, w3_s, sems.at[12])
    cp_w4 = pltpu.make_async_copy(w4_hbm, w4_s, sems.at[13])

    cp_x3.start()
    for c in cp_w0:
        c.start()
    for c in range(1, NKC):
        cp_w(wk_hbm, IK, c).start()
    for c in range(NKC):
        cp_w(wv_hbm, IV, c).start()

    def relayout_piece(j, p, q):
        wi = st.bitcast(jnp.int32)
        sub = wi.at[pl.ds(pl.multiple_of((j % 8) * (DC * 16), DC * 16), DC * 16), :]
        n = DC // RP
        dr = pl.multiple_of((j % NKC) * (DC // 2) + q * (n // 2), n // 2)
        hb0 = (j // NKC) * H
        w = sub[pl.ds(p + q * n * 16, n, stride=16), :]
        lo = jax.lax.bitcast_convert_type(w << 16, F32).astype(BF16)
        hi = jax.lax.bitcast_convert_type(w & np.int32(-65536), F32).astype(BF16)
        w_s[hb0 + 2 * p, pl.ds(dr, n // 2), :] = pltpu.bitcast(lo, jnp.int32)
        w_s[hb0 + 2 * p + 1, pl.ds(dr, n // 2), :] = pltpu.bitcast(hi, jnp.int32)

    def wtile(m, h):
        return pltpu.bitcast(w_s[m * H + h], BF16)

    hb[S:S + PAD, :] = jnp.zeros((PAD, D), F32)

    with jax.named_scope('S_p0'):
        cp_x3.wait()
        for g in range(4):
            y = _ln(jnp.concatenate([xr[16 * g + s].astype(F32) for s in range(16)], axis=0))
            y = y.astype(BF16)
            for kc in range(NKC):
                xo[kc, g * 128:(g + 1) * 128, :] = y[:, kc * DC:(kc + 1) * DC]
        for q in range(RP // 2 if HALF else RP):
            cp_w0[q].wait()
            for p in range(H // 2):
                relayout_piece(0, p, q)

    RS = 128
    items = [(h, r) for h in range(H) for r in range(0, 512, RS)]

    def proj_first():
        cp_w(wq_hbm, IQ, 0).start()
        n = len(items)

        def run(k0, kn, accumulate, t0, waits, pieces):
            for t, (h, r) in enumerate(items):
                w = pltpu.bitcast(w_s[h, k0 // 2:(k0 + kn) // 2, :], BF16)
                res = _dot(xo[0, r:r + RS, k0:k0 + kn], w)
                if t == t0:
                    for c in waits:
                        c()
                if t >= t0:
                    for pc in pieces[(t - t0) * len(pieces) // (n - t0):
                                     (t + 1 - t0) * len(pieces) // (n - t0)]:
                        relayout_piece(*pc)
                if accumulate:
                    res = res + acc[h, r:r + RS, :]
                acc[h, r:r + RS, :] = res

        next_pieces = [(1, p, q) for p in range(H // 2) for q in range(RP)]
        if HALF:
            run(0, DC // 2, False, T0A, [cp_w0[2].wait, cp_w0[3].wait],
                [(0, p, q) for q in (2, 3) for p in range(H // 2)])
            run(DC // 2, DC // 2, True, T0B, [lambda: wait_w(1)], next_pieces)
        else:
            run(0, DC, False, n // 2, [lambda: wait_w(1)], next_pieces)

    def proj(j, carry):
        @pl.when(j < NKC)
        def _():
            cp_w(wq_hbm, IQ, j).start()

        @pl.when(j == NKC)
        def _():
            cp_x.start()
            for c in cp_wo:
                c.start()

        @pl.when(j < 11)
        def _():
            wait_w(j + 1)

        jn = jnp.minimum(j + 1, 11)
        kc = j % NKC
        hb0 = (j // NKC) * H
        dr = pl.multiple_of(kc * (DC // 2), DC // 2)
        first = kc == 0
        for t, (h, r) in enumerate(items):
            w = pltpu.bitcast(w_s[hb0 + h, pl.ds(dr, DC // 2), :], BF16)
            res = _dot(xo[kc, r:r + RS, :], w)
            if t % 2 == 1:
                p, q = divmod(t // 2, RP)
                relayout_piece(jn, p, q)
            new = res + jnp.where(first, 0.0, acc[h, r:r + RS, :])
            acc[h, r:r + RS, :] = new
            qkvo[hb0 + h, r:r + RS, :] = new.astype(BF16)
        return carry

    with jax.named_scope('S_proj'):
        if PEEL_PROJ:
            proj_first()
        jax.lax.fori_loop(PEEL_PROJ, 12, proj, 0, unroll=PROJ_UNROLL)

    cp_w1.start()
    cp_w2.start()
    cp_w3.start()
    cp_w4.start()
    cp_x.wait()
    xn[0:24, :] = _ln(gb[PAD:PAD + SEG, :].astype(F32)[0:24])
    for c in cp_wo:
        c.wait()

    L = M + SEG
    c_exp = (E ** -0.5) * 1.4426950408889634

    def step(i, mem):
        r0 = pl.multiple_of(i * SEG, SEG)
        r8 = pl.multiple_of(i * 8, 8)
        lhs = jnp.concatenate([mem, xn[pl.ds(r0, 24), :]], axis=0).astype(BF16)
        row = jax.lax.broadcasted_iota(jnp.int32, (L, L), 0)
        col = jax.lax.broadcasted_iota(jnp.int32, (L, L), 1)
        mask = (row < M) | (row >= col)

        rn = pl.multiple_of(jnp.minimum(i + 1, NSEG - 1) * SEG, SEG)
        xn_next = _ln(gb[pl.ds(PAD + rn, SEG), :].astype(F32)[0:24])

        qkv, sc, av, oh = {}, {}, {}, {}
        acc_o = []

        def st_proj(h):
            qkv[h] = tuple(
                jnp.concatenate([_dot(lhs, wtile(m, h)),
                                 qkvo[m * H + h, pl.ds(r8, 8), :].astype(F32)], axis=0)
                for m in (IQ, IK, IV))

        def st_score(h):
            s = jax.lax.dot_general(qkv[h][0], qkv[h][1], (((1,), (1,)), ((), ())),
                                    preferred_element_type=F32)
            s = jnp.where(mask, s, -1e30)
            sc[h] = (s, jnp.max(s, axis=-1, keepdims=True))

        def st_pv(h):
            s, mx = sc.pop(h)
            p = jnp.exp2((s - mx) * c_exp)
            av[h] = (_dot(p, qkv.pop(h)[2]), jnp.sum(p, axis=-1, keepdims=True))

        def st_norm(h):
            o, l = av.pop(h)
            r = pl.reciprocal(l, approx=True)
            r = r * (2.0 - l * r)
            o = o * r
            oh[h] = o[0:32].astype(BF16)
            oo[h, pl.ds(r8, 8), :] = o[32:40].astype(BF16)

        def st_out(h):
            w = jnp.concatenate([wo_s[n, h * E:(h + 1) * E, :] for n in range(NT)], axis=1)
            r = _dot(oh.pop(h), w)
            acc_o[:] = [r if not acc_o else acc_o[0] + r]

        stages = tuple(zip((st_proj, st_score, st_pv, st_norm, st_out), LAGS))
        for t in range(H + stages[-1][1]):
            for fn, lag in stages:
                if 0 <= t - lag < H:
                    fn(t - lag)

        xn[pl.ds(rn, 24), :] = xn_next
        res = acc_o[0]
        xv = gb[pl.ds(PAD + r0, SEG), :].astype(F32)
        hb[pl.ds(r0, SEG), :] = jnp.concatenate([xv[0:24] + res[8:32], xv[24:32]], axis=0)
        return res[0:8]

    with jax.named_scope('S_rec'):
        jax.lax.fori_loop(0, NSEG, step, mem0_ref[...].astype(F32), unroll=REC_UNROLL)

    def tail_out(c, carry):
        r = pl.multiple_of(c * 128, 128)
        lhs = jnp.concatenate([oo[h, pl.ds(r, 128), :] for h in range(H)], axis=1)
        for n in range(NT):
            res = _dot(lhs, wo_s[n])
            cs = slice(n * 128, (n + 1) * 128)
            for s in range(16):
                rr = pl.multiple_of(c * (16 * SEG) + s * SEG + 24, 8)
                hb[pl.ds(rr, 8), cs] = hb[pl.ds(rr, 8), cs] + res[8 * s:8 * s + 8]
        return carry

    with jax.named_scope('S_tailout'):
        jax.lax.fori_loop(0, 4, tail_out, 0)

    cp_w1.wait()
    cp_w2.wait()
    cp_w3.wait()
    cp_w4.wait()
    gb[0:PAD, :] = jnp.zeros((PAD, D), BF16)
    yb = xn

    def norm1(r, n):
        y = _ln(hb[pl.ds(r, n), :])
        yb[pl.ds(r, n), :] = y
        return _ln(y).astype(BF16)

    def mix1(z, r, n):
        gb[pl.ds(r + PAD, n), :] = _gelu(_dot(z, w1_s[...])).astype(BF16)

    def shifted(r):
        c = D // 4
        parts = []
        for gi, sh in enumerate((-1, 1, -2, 2)):
            win = gb[pl.ds(r, RB + 2 * PAD), gi * c:(gi + 1) * c].astype(F32)
            parts.append(win[PAD + sh:PAD + sh + RB].astype(BF16))
        return jnp.concatenate(parts, axis=1)

    def mlp_out(b, r, x1):
        z2 = _ln(x1).astype(BF16)
        acc = hb[pl.ds(r, RB), :] + x1
        nf = FF // FC
        for f in range(nf):
            a = _gelu(_dot(z2, w3_s[:, f * FC:(f + 1) * FC])).astype(BF16)
            if f < nf - 1 or not OC:
                acc = acc + _dot(a, w4_s[f * FC:(f + 1) * FC, :])
            else:
                for c in range(0, D, OC):
                    o = acc[:, c:c + OC] + _dot(a, w4_s[f * FC:(f + 1) * FC, c:c + OC])
                    outb[pl.ds(r, RB), c:c + OC] = o.astype(BF16)
        if not OC:
            outb[pl.ds(r, RB), :] = acc.astype(BF16)
        pltpu.make_async_copy(outb.at[pl.ds(r, RB), :], out_hbm.at[pl.ds(r, RB), :],
                              osems.at[b]).start()

    with jax.named_scope('S_pro'):
        mix1(norm1(0, RB + PAD), 0, RB + PAD)

    def mlp(b, carry):
        r = pl.multiple_of(b * RB, RB)
        rn = pl.multiple_of(jnp.minimum(b + 1, NRB - 1) * RB + PAD, PAD)
        if ORDER == 0:
            gs = shifted(r)
            x1 = yb[pl.ds(r, RB), :] + _dot(gs, w2_s[...])
            z = norm1(rn, RB)
        elif ORDER == 1:
            gs = shifted(r)
            z = norm1(rn, RB)
            x1 = yb[pl.ds(r, RB), :] + _dot(gs, w2_s[...])
        elif ORDER == 2:
            z = norm1(rn, RB)
            gs = shifted(r)
            x1 = yb[pl.ds(r, RB), :] + _dot(gs, w2_s[...])
        elif ORDER == 3:
            gs = shifted(r)
            xa = yb[pl.ds(r, RB), 0:HS] + _dot(gs, w2_s[:, 0:HS])
            z = norm1(rn, RB)
            xb = yb[pl.ds(r, RB), HS:D] + _dot(gs, w2_s[:, HS:D])
            x1 = jnp.concatenate([xa, xb], axis=1)
        mix1(z, rn, RB)
        mlp_out(b, r, x1)
        return carry

    with jax.named_scope('S_mlp'):
        jax.lax.fori_loop(0, NRB, mlp, 0)

    for b in range(NRB):
        pltpu.make_async_copy(outb.at[pl.ds(b * RB, RB), :], out_hbm.at[pl.ds(b * RB, RB), :],
                              osems.at[b]).wait()


@functools.partial(jax.jit, static_argnames=("A_seg_len",))
def pallas_sequential_preLN__memory_aug_recurrent_mem_tr__mixer_s_mlp__prompt_kernel(
    A_x: jax.Array,
    A_mem0: jax.Array,
    A_Wq: jax.Array,
    A_Wk: jax.Array,
    A_Wv: jax.Array,
    A_Wo: jax.Array,
    A_seg_len: int,
    B_x: jax.Array,
    B_w1: jax.Array,
    B_w2: jax.Array,
    B_w3: jax.Array,
    B_w4: jax.Array,
):
    assert A_seg_len == SEG
    assert A_x.shape == (1, S, D) and A_mem0.shape == (1, M, D) and A_Wq.shape == (D, H, E)
    any_spec = pl.BlockSpec(memory_space=pl.ANY)
    vm = pltpu.VMEM
    out = pl.pallas_call(
        _kernel,
        out_shape=jax.ShapeDtypeStruct((S, D), A_x.dtype),
        in_specs=[any_spec, any_spec, pl.BlockSpec(memory_space=pltpu.VMEM)] + [any_spec] * 8,
        out_specs=any_spec,
        scratch_shapes=[
            vm((3 * H, D // 2, E), jnp.int32),
            vm((NT, H * E, 128), BF16),
            vm((8 * (D // 4) * H, E), BF16),
            vm((H, 512, E), F32),
            vm((S + PAD, D), F32), vm((S + PAD, D), F32),
            vm((NSEG, 8, D), BF16),
            vm((4, 512, D // 4), BF16),
            vm((3 * H, 512, E), BF16),
            vm((H, 512, E), BF16),
            vm((D, D), BF16), vm((D, D), BF16), vm((D, FF), BF16), vm((FF, D), BF16),
            vm((S + 2 * PAD, D), BF16),
            vm((S, D), BF16),
            pltpu.SemaphoreType.DMA((16 + 13 + 4,)),
            pltpu.SemaphoreType.DMA((NRB,)),
        ],
        compiler_params=pltpu.CompilerParams(vmem_limit_bytes=122 * 2 ** 20),
    )(A_x.reshape(S, D), A_x.reshape(NSEG, SEG, D), A_mem0.reshape(M, D),
      A_Wq.reshape(D * H, E), A_Wk.reshape(D * H, E), A_Wv.reshape(D * H, E),
      A_Wo.reshape(H * E, D), B_w1, B_w2, B_w3, B_w4)
    return out.reshape(1, S, D)
```

```python
import functools

import jax
import jax.numpy as jnp
import numpy as np
import jax.experimental.pallas as pl
import jax.experimental.pallas.tpu as pltpu

F32 = jnp.float32
BF16 = jnp.bfloat16

S = 2048
D = 1024
H = 32
E = 128
M = 8
SEG = 32
NSEG = S // SEG
FF = 3584
NT = D // 128
EPS = 1e-5
PAD = 16
RB = 128
NRB = S // RB
FC = 896
REC_UNROLL = 2
LAGS = (0, 18, 26, 28, 32)


def _ln(x):
    m = jnp.mean(x, axis=-1, keepdims=True)
    c = x - m
    v = jnp.mean(c * c, axis=-1, keepdims=True)
    return c * jax.lax.rsqrt(v + EPS)


def _gelu(x):
    return jax.nn.gelu(x, approximate=True)


def _dot(a, b):
    return jnp.dot(a, b, preferred_element_type=F32)


def _kernel(x_hbm, x3_hbm, mem0_ref, wq_hbm, wk_hbm, wv_hbm, wo_hbm, w1_hbm, w2_hbm, w3_hbm, w4_hbm,
            out_hbm,
            w_s, wo_s, st, acc, xn, hb, xr, xo, qkvo, oo,
            w1_s, w2_s, w3_s, w4_s, gb, outb, sems, osems):
    NKC = 4
    DC = D // NKC
    IK, IV, IQ = 0, 1, 2

    cp_x3 = pltpu.make_async_copy(x3_hbm.at[:, pl.ds(24, 8), :], xr, sems.at[0])

    RP = 4
    NC = DC * H
    NP = NC // RP
    WB = 16

    def cp_w(src, m, c):
        slot = (m * NKC + c) % 8
        return pltpu.make_async_copy(src.at[pl.ds(pl.multiple_of(c * NC, NC), NC), :],
                                     st.at[pl.ds(pl.multiple_of(slot * NC, NC), NC), :],
                                     sems.at[WB + m * NKC + c])

    cp_w0 = [pltpu.make_async_copy(wk_hbm.at[pl.ds(q * NP, NP), :], st.at[pl.ds(q * NP, NP), :],
                                   sems.at[WB + 13 + q]) for q in range(RP)]

    def wait_w(j):
        r = pl.multiple_of((j % 8) * NC, NC)
        pltpu.make_async_copy(st.at[pl.ds(r, NC), :], st.at[pl.ds(r, NC), :],
                              sems.at[WB + j]).wait()

    cp_x = pltpu.make_async_copy(x_hbm, gb.at[pl.ds(PAD, S), :], sems.at[1])

    cp_wo = [pltpu.make_async_copy(wo_hbm.at[:, pl.ds(n * 128, 128)], wo_s.at[n], sems.at[2 + n])
             for n in range(NT)]
    cp_w1 = pltpu.make_async_copy(w1_hbm, w1_s, sems.at[10])
    cp_w2 = pltpu.make_async_copy(w2_hbm, w2_s, sems.at[11])
    cp_w3 = pltpu.make_async_copy(w3_hbm, w3_s, sems.at[12])
    cp_w4 = pltpu.make_async_copy(w4_hbm, w4_s, sems.at[13])

    cp_x3.start()
    for c in cp_w0:
        c.start()
    for c in range(1, NKC):
        cp_w(wk_hbm, IK, c).start()
    for c in range(NKC):
        cp_w(wv_hbm, IV, c).start()

    def relayout_piece(j, p, q):
        wi = st.bitcast(jnp.int32)
        sub = wi.at[pl.ds(pl.multiple_of((j % 8) * (DC * 16), DC * 16), DC * 16), :]
        n = DC // RP
        dr = pl.multiple_of((j % NKC) * (DC // 2) + q * (n // 2), n // 2)
        hb0 = (j // NKC) * H
        w = sub[pl.ds(p + q * n * 16, n, stride=16), :]
        lo = jax.lax.bitcast_convert_type(w << 16, F32).astype(BF16)
        hi = jax.lax.bitcast_convert_type(w & np.int32(-65536), F32).astype(BF16)
        w_s[hb0 + 2 * p, pl.ds(dr, n // 2), :] = pltpu.bitcast(lo, jnp.int32)
        w_s[hb0 + 2 * p + 1, pl.ds(dr, n // 2), :] = pltpu.bitcast(hi, jnp.int32)

    def wtile(m, h):
        return pltpu.bitcast(w_s[m * H + h], BF16)

    hb[S:S + PAD, :] = jnp.zeros((PAD, D), F32)

    with jax.named_scope('S_p0'):
        cp_x3.wait()
        for g in range(4):
            y = _ln(jnp.concatenate([xr[16 * g + s].astype(F32) for s in range(16)], axis=0))
            y = y.astype(BF16)
            for kc in range(NKC):
                xo[kc, g * 128:(g + 1) * 128, :] = y[:, kc * DC:(kc + 1) * DC]
        for q in range(RP // 2):
            cp_w0[q].wait()
            for p in range(H // 2):
                relayout_piece(0, p, q)

    RS = 128
    items = [(h, r) for h in range(H) for r in range(0, 512, RS)]

    def proj_first():
        n = len(items)

        def run(k0, kn, accumulate, t0, waits, pieces):
            for t, (h, r) in enumerate(items):
                w = pltpu.bitcast(w_s[h, k0 // 2:(k0 + kn) // 2, :], BF16)
                res = _dot(xo[0, r:r + RS, k0:k0 + kn], w)
                if t == t0:
                    for c in waits:
                        c()
                if t >= t0:
                    for pc in pieces[(t - t0) * len(pieces) // (n - t0):
                                     (t + 1 - t0) * len(pieces) // (n - t0)]:
                        relayout_piece(*pc)
                if accumulate:
                    res = res + acc[h, r:r + RS, :]
                acc[h, r:r + RS, :] = res

        next_pieces = [(1, p, q) for p in range(H // 2) for q in range(RP)]
        run(0, DC // 2, False, n // 2, [cp_w0[2].wait, cp_w0[3].wait],
            [(0, p, q) for q in (2, 3) for p in range(H // 2)])
        cp_w(wq_hbm, IQ, 0).start()
        run(DC // 2, DC // 2, True, n // 2, [lambda: wait_w(1)], next_pieces)

    def proj(j, carry):
        @pl.when(j < NKC)
        def _():
            cp_w(wq_hbm, IQ, j).start()

        @pl.when(j == NKC)
        def _():
            cp_x.start()
            for c in cp_wo:
                c.start()

        @pl.when(j < 11)
        def _():
            wait_w(j + 1)

        jn = jnp.minimum(j + 1, 11)
        kc = j % NKC
        hb0 = (j // NKC) * H
        dr = pl.multiple_of(kc * (DC // 2), DC // 2)
        first = kc == 0
        for t, (h, r) in enumerate(items):
            w = pltpu.bitcast(w_s[hb0 + h, pl.ds(dr, DC // 2), :], BF16)
            res = _dot(xo[kc, r:r + RS, :], w)
            if t % 2 == 1:
                p, q = divmod(t // 2, RP)
                relayout_piece(jn, p, q)
            new = res + jnp.where(first, 0.0, acc[h, r:r + RS, :])
            acc[h, r:r + RS, :] = new
            qkvo[hb0 + h, r:r + RS, :] = new.astype(BF16)
        return carry

    with jax.named_scope('S_proj'):
        proj_first()
        jax.lax.fori_loop(1, 3 * NKC, proj, 0)

    cp_w1.start()
    cp_w2.start()
    cp_w3.start()
    cp_w4.start()
    cp_x.wait()
    xn[0:24, :] = _ln(gb[PAD:PAD + SEG, :].astype(F32)[0:24])
    for c in cp_wo:
        c.wait()

    L = M + SEG
    c_exp = (E ** -0.5) * 1.4426950408889634

    def step(i, mem):
        r0 = pl.multiple_of(i * SEG, SEG)
        r8 = pl.multiple_of(i * 8, 8)
        lhs = jnp.concatenate([mem, xn[pl.ds(r0, 24), :]], axis=0).astype(BF16)
        row = jax.lax.broadcasted_iota(jnp.int32, (L, L), 0)
        col = jax.lax.broadcasted_iota(jnp.int32, (L, L), 1)
        mask = (row < M) | (row >= col)

        rn = pl.multiple_of(jnp.minimum(i + 1, NSEG - 1) * SEG, SEG)
        xn_next = _ln(gb[pl.ds(PAD + rn, SEG), :].astype(F32)[0:24])

        qkv, sc, av, oh = {}, {}, {}, {}
        acc_o = []

        def st_proj(h):
            qkv[h] = tuple(
                jnp.concatenate([_dot(lhs, wtile(m, h)),
                                 qkvo[m * H + h, pl.ds(r8, 8), :].astype(F32)], axis=0)
                for m in (IQ, IK, IV))

        def st_score(h):
            s = jax.lax.dot_general(qkv[h][0], qkv[h][1], (((1,), (1,)), ((), ())),
                                    preferred_element_type=F32)
            s = jnp.where(mask, s, -1e30)
            sc[h] = (s, jnp.max(s, axis=-1, keepdims=True))

        def st_pv(h):
            s, mx = sc.pop(h)
            p = jnp.exp2((s - mx) * c_exp)
            av[h] = (_dot(p, qkv.pop(h)[2]), jnp.sum(p, axis=-1, keepdims=True))

        def st_norm(h):
            o, l = av.pop(h)
            r = pl.reciprocal(l, approx=True)
            r = r * (2.0 - l * r)
            o = o * r
            oh[h] = o[0:32].astype(BF16)
            oo[h, pl.ds(r8, 8), :] = o[32:40].astype(BF16)

        def st_out(h):
            w = jnp.concatenate([wo_s[n, h * E:(h + 1) * E, :] for n in range(NT)], axis=1)
            r = _dot(oh.pop(h), w)
            acc_o[:] = [r if not acc_o else acc_o[0] + r]

        stages = tuple(zip((st_proj, st_score, st_pv, st_norm, st_out), LAGS))
        for t in range(H + stages[-1][1]):
            for fn, lag in stages:
                if 0 <= t - lag < H:
                    fn(t - lag)

        xn[pl.ds(rn, 24), :] = xn_next
        res = acc_o[0]
        xv = gb[pl.ds(PAD + r0, SEG), :].astype(F32)
        hb[pl.ds(r0, SEG), :] = jnp.concatenate([xv[0:24] + res[8:32], xv[24:32]], axis=0)
        return res[0:8]

    with jax.named_scope('S_rec'):
        jax.lax.fori_loop(0, NSEG, step, mem0_ref[...].astype(F32), unroll=REC_UNROLL)

    def tail_out(c, carry):
        r = pl.multiple_of(c * 128, 128)
        lhs = jnp.concatenate([oo[h, pl.ds(r, 128), :] for h in range(H)], axis=1)
        for n in range(NT):
            res = _dot(lhs, wo_s[n])
            cs = slice(n * 128, (n + 1) * 128)
            for s in range(16):
                rr = pl.multiple_of(c * (16 * SEG) + s * SEG + 24, 8)
                hb[pl.ds(rr, 8), cs] = hb[pl.ds(rr, 8), cs] + res[8 * s:8 * s + 8]
        return carry

    with jax.named_scope('S_tailout'):
        jax.lax.fori_loop(0, 4, tail_out, 0)

    cp_w1.wait()
    cp_w2.wait()
    cp_w3.wait()
    cp_w4.wait()
    gb[0:PAD, :] = jnp.zeros((PAD, D), BF16)
    yb = xn

    def norm1(r, n):
        y = _ln(hb[pl.ds(r, n), :])
        yb[pl.ds(r, n), :] = y
        return _ln(y).astype(BF16)

    def mix1(z, r, n):
        gb[pl.ds(r + PAD, n), :] = _gelu(_dot(z, w1_s[...])).astype(BF16)

    def shifted(r):
        c = D // 4
        parts = []
        for gi, sh in enumerate((-1, 1, -2, 2)):
            win = gb[pl.ds(r, RB + 2 * PAD), gi * c:(gi + 1) * c].astype(F32)
            parts.append(win[PAD + sh:PAD + sh + RB].astype(BF16))
        return jnp.concatenate(parts, axis=1)

    def mlp_out(b, r, x1):
        z2 = _ln(x1).astype(BF16)
        acc = hb[pl.ds(r, RB), :] + x1
        for f in range(FF // FC):
            a = _gelu(_dot(z2, w3_s[:, f * FC:(f + 1) * FC])).astype(BF16)
            acc = acc + _dot(a, w4_s[f * FC:(f + 1) * FC, :])
        outb[pl.ds(r, RB), :] = acc.astype(BF16)
        pltpu.make_async_copy(outb.at[pl.ds(r, RB), :], out_hbm.at[pl.ds(r, RB), :],
                              osems.at[b]).start()

    with jax.named_scope('S_pro'):
        mix1(norm1(0, RB + PAD), 0, RB + PAD)

    def mlp(b, carry):
        r = pl.multiple_of(b * RB, RB)
        rn = pl.multiple_of(jnp.minimum(b + 1, NRB - 1) * RB + PAD, PAD)
        gs = shifted(r)
        z = norm1(rn, RB)
        x1 = yb[pl.ds(r, RB), :] + _dot(gs, w2_s[...])
        mix1(z, rn, RB)
        mlp_out(b, r, x1)
        return carry

    with jax.named_scope('S_mlp'):
        jax.lax.fori_loop(0, NRB, mlp, 0)

    for b in range(NRB):
        pltpu.make_async_copy(outb.at[pl.ds(b * RB, RB), :], out_hbm.at[pl.ds(b * RB, RB), :],
                              osems.at[b]).wait()


@functools.partial(jax.jit, static_argnames=("A_seg_len",))
def pallas_sequential_preLN__memory_aug_recurrent_mem_tr__mixer_s_mlp__prompt_kernel(
    A_x: jax.Array,
    A_mem0: jax.Array,
    A_Wq: jax.Array,
    A_Wk: jax.Array,
    A_Wv: jax.Array,
    A_Wo: jax.Array,
    A_seg_len: int,
    B_x: jax.Array,
    B_w1: jax.Array,
    B_w2: jax.Array,
    B_w3: jax.Array,
    B_w4: jax.Array,
):
    assert A_seg_len == SEG
    assert A_x.shape == (1, S, D) and A_mem0.shape == (1, M, D) and A_Wq.shape == (D, H, E)
    any_spec = pl.BlockSpec(memory_space=pl.ANY)
    vm = pltpu.VMEM
    out = pl.pallas_call(
        _kernel,
        out_shape=jax.ShapeDtypeStruct((S, D), A_x.dtype),
        in_specs=[any_spec, any_spec, pl.BlockSpec(memory_space=pltpu.VMEM)] + [any_spec] * 8,
        out_specs=any_spec,
        scratch_shapes=[
            vm((3 * H, D // 2, E), jnp.int32),
            vm((NT, H * E, 128), BF16),
            vm((8 * (D // 4) * H, E), BF16),
            vm((H, 512, E), F32),
            vm((S + PAD, D), F32), vm((S + PAD, D), F32),
            vm((NSEG, 8, D), BF16),
            vm((4, 512, D // 4), BF16),
            vm((3 * H, 512, E), BF16),
            vm((H, 512, E), BF16),
            vm((D, D), BF16), vm((D, D), BF16), vm((D, FF), BF16), vm((FF, D), BF16),
            vm((S + 2 * PAD, D), BF16),
            vm((S, D), BF16),
            pltpu.SemaphoreType.DMA((16 + 13 + 4,)),
            pltpu.SemaphoreType.DMA((NRB,)),
        ],
        compiler_params=pltpu.CompilerParams(vmem_limit_bytes=122 * 2 ** 20),
    )(A_x.reshape(S, D), A_x.reshape(NSEG, SEG, D), A_mem0.reshape(M, D),
      A_Wq.reshape(D * H, E), A_Wk.reshape(D * H, E), A_Wv.reshape(D * H, E),
      A_Wo.reshape(H * E, D), B_w1, B_w2, B_w3, B_w4)
    return out.reshape(1, S, D)
```
